```python
import jax
import jax.numpy as jnp

def _softmax(x, axis=-1):
    return jax.nn.softmax(x, axis=axis)
def _gelu(x):
    return jax.nn.gelu(x, approximate=True)
def _silu(x):
    return jax.nn.silu(x)
def _sigmoid(x):
    return jax.nn.sigmoid(x)
def _layernorm(x, axis=-1, eps=1e-5):
    m = jnp.mean(x, axis=axis, keepdims=True)
    v = jnp.var(x, axis=axis, keepdims=True)
    return (x - m) / jnp.sqrt(v + eps)
def _scatter_add(tgt, idx, src, axis=0):
    return tgt.at[idx].add(src)
def _segment_sum(src, seg, n):
    return jax.ops.segment_sum(src, seg, n)
class _Rng:
    def __init__(self, key):
        self._k = key
    def _next(self):
        self._k, sub = jax.random.split(self._k)
        return sub
    def normal(self, shape):
        return jax.random.normal(self._next(), shape, dtype=jnp.bfloat16)
    def randint(self, lo, hi, shape):
        return jax.random.randint(self._next(), shape, lo, hi, dtype=jnp.int32)
    def uniform(self, shape, lo=0.0, hi=1.0):
        return jax.random.uniform(self._next(), shape, jnp.bfloat16, lo, hi)
    def permutation(self, n):
        return jax.random.permutation(self._next(), n)


kernel_name = 'concat_heads__mha_block_cached__compressed_kv_cla__decode'

def setup_inputs():
    _rng = _Rng(jax.random.key(int.from_bytes(__import__("os").urandom(4), "little")))
    _w = (lambda a: (lambda t: t.astype(jnp.bfloat16) if jnp.issubdtype(t.dtype, jnp.floating) else t)(jnp.asarray(a)))
    def _A_setup():
        B, Sq, D = 4, 1, 576
        H, Sk, Dh = 32, 4096, 128
        return {
            "x": _w((lambda *s: _rng.normal(s) * 0.05)(B, Sq, D)),
            "k_cache": _w((lambda *s: _rng.normal(s) * 0.05)(B, H, Sk, Dh)),
            "v_cache": _w((lambda *s: _rng.normal(s) * 0.05)(B, H, Sk, Dh)),
            "wq": _w((lambda *s: _rng.normal(s) * 0.05)(D, H * Dh) * (D ** -0.5)),
            "wo": _w((lambda *s: _rng.normal(s) * 0.05)(H * Dh, D) * ((H * Dh) ** -0.5)),
        }
    _A_in = _A_setup()

    def _B_setup():
        B, H, Sq, Sk, D, M = 4, 32, 1, 4096, 128, 576
        Dc = 4 * D
        return {
            "x": _w((lambda *s: _rng.normal(s) * 0.05)(B, Sq, M)),
            "c_kv": _w((lambda *s: _rng.normal(s) * 0.05)(B, Sk, Dc)),
            "w_q": _w((lambda *s: _rng.normal(s) * 0.05)(M, H, D) * (M ** -0.5)),
            "w_uk": _w((lambda *s: _rng.normal(s) * 0.05)(Dc, H, D) * (Dc ** -0.5)),
            "w_uv": _w((lambda *s: _rng.normal(s) * 0.05)(Dc, H, D) * (Dc ** -0.5)),
            "w_o": _w((lambda *s: _rng.normal(s) * 0.05)(H, D, M) * ((H * D) ** -0.5)),
        }
    _B_in = _B_setup()

    return {
        "A_x": _A_in["x"],
        "A_k_cache": _A_in["k_cache"],
        "A_v_cache": _A_in["v_cache"],
        "A_wq": _A_in["wq"],
        "A_wo": _A_in["wo"],
        "B_x": _B_in["x"],
        "B_c_kv": _B_in["c_kv"],
        "B_w_q": _B_in["w_q"],
        "B_w_uk": _B_in["w_uk"],
        "B_w_uv": _B_in["w_uv"],
        "B_w_o": _B_in["w_o"],
    }

def reference(A_x, A_k_cache, A_v_cache, A_wq, A_wo, B_x, B_c_kv, B_w_q, B_w_uk, B_w_uv, B_w_o):
    def _A_ref(x, k_cache, v_cache, wq, wo):
        B, Sq, D = x.shape
        H, Dh = 32, 128
        q = (lambda x, *d: x.transpose(*d))((x @ wq).reshape(B, Sq, H, Dh), 0, 2, 1, 3)
        scores = jnp.einsum("bhqd,bhkd->bhqk", q, k_cache) * (Dh ** -0.5)
        p = _softmax(scores, axis=-1)
        o = jnp.einsum("bhqk,bhkd->bhqd", p, v_cache)
        return (lambda x, *d: x.transpose(*d))(o, 0, 2, 1, 3).reshape(B, Sq, H * Dh) @ wo

    def _B_ref(x, c_kv, w_q, w_uk, w_uv, w_o):
        B, Sq, M = x.shape[0], x.shape[1], x.shape[2]
        Sk = c_kv.shape[1]
        H, D = w_q.shape[1], w_q.shape[2]
        q = jnp.einsum("bqm,mhd->bhqd", x, w_q)
        k = jnp.einsum("bkc,chd->bhkd", c_kv, w_uk)
        v = jnp.einsum("bkc,chd->bhkd", c_kv, w_uv)
        scores = jnp.einsum("bhqd,bhkd->bhqk", q, k) * (D ** -0.5)
        off = Sk - Sq
        qi = jnp.arange(Sq)[:, None]
        kj = jnp.arange(Sk)[None, :]
        cmask = kj <= (qi + off)
        scores = jnp.where(cmask[None, None], scores, -1e9)
        p = _softmax(scores, axis=-1)
        ctx = jnp.einsum("bhqk,bhkd->bhqd", p, v)
        return jnp.einsum("bhqd,hdm->bqm", ctx, w_o)

    a = _A_ref(A_x, A_k_cache, A_v_cache, A_wq, A_wo)
    b = _B_ref(B_x, B_c_kv, B_w_q, B_w_uk, B_w_uv, B_w_o)
    return jnp.concatenate([a, b], axis=-1)
```

```python
import functools

import jax
import jax.numpy as jnp
from jax import lax
import jax.experimental.pallas as pl
import jax.experimental.pallas.tpu as pltpu

_F32 = jnp.float32
_BF16 = jnp.bfloat16
_ROWS = 8
_RING = 8
_KC = 512


def _dot(a, b):
    return lax.dot_general(a, b, (((1,), (0,)), ((), ())), preferred_element_type=_F32)


def _dot_nt(a, b):
    return lax.dot_general(a, b, (((1,), (1,)), ((), ())), preferred_element_type=_F32)


def _head_pair(w_ref, j, rows, heads):
    w = w_ref.bitcast(jnp.uint32)[pl.ds(j, rows, stride=heads // 2), :]
    lo = lax.bitcast_convert_type(w << 16, _F32).astype(_BF16)
    hi = lax.bitcast_convert_type((w >> 16) << 16, _F32).astype(_BF16)
    return lo, hi


def _pad_rows(x):
    x = x.astype(_F32)
    pad = jnp.zeros((_ROWS - x.shape[0], x.shape[1]), _F32)
    return jnp.concatenate([x, pad], axis=0).astype(_BF16)


def _kernel(xa_hbm, k_hbm, v_hbm, wqa_hbm, woa_hbm,
            xb_hbm, c_hbm, wqb_hbm, wuk_hbm, wuv_hbm, wob_hbm,
            out_ref,
            xa_v, xb_v, kbuf, vbuf, wqa_v, woa_v, c_v, wqb_v, wuk_v, wuv_v, wob_v,
            qa_s, qb_s, lat_s, bat_s, sc_s, o_s, acc_s,
            ksem, vsem, csem, wsem):
    nb, nh, sk, dh = k_hbm.shape
    dm = xa_hbm.shape[1]
    dc = c_hbm.shape[2]
    ncc = dc // 128
    nsteps = nb * nh
    scale = dh ** -0.5

    def k_copy(i):
        slot = i % _RING
        return pltpu.make_async_copy(k_hbm.at[i % nb, i // nb], kbuf.at[slot], ksem.at[slot])

    def v_copy(i):
        slot = i % _RING
        return pltpu.make_async_copy(v_hbm.at[i % nb, i // nb], vbuf.at[slot], vsem.at[slot])

    def c_copy(b):
        return pltpu.make_async_copy(c_hbm.at[b], c_v.at[b], csem.at[b])

    whole = {
        "xa": (xa_hbm, xa_v, 0), "xb": (xb_hbm, xb_v, 1),
        "wqb": (wqb_hbm, wqb_v, 2), "wuk": (wuk_hbm, wuk_v, 3),
        "wuv": (wuv_hbm, wuv_v, 4), "wob": (wob_hbm, wob_v, 5),
        "wqa": (wqa_hbm, wqa_v, 6), "woa": (woa_hbm, woa_v, 7),
    }

    def w_copy(name):
        src, dst, s = whole[name]
        return pltpu.make_async_copy(src, dst, wsem.at[s])

    w_copy("wqb").start()
    w_copy("xb").start(priority=1)
    w_copy("xa").start(priority=1)
    w_copy("wuk").start(priority=1)
    for b in range(nb):
        c_copy(b).start(priority=b % 2)
    w_copy("wuv").start()
    w_copy("wob").start(priority=1)
    w_copy("wqa").start()
    w_copy("woa").start(priority=1)
    for i in range(_RING):
        k_copy(i).start()
        v_copy(i).start(priority=1)

    w_copy("xb").wait()
    w_copy("wqb").wait()
    xb = _pad_rows(xb_v[...])

    for j in range(nh // 2):
        for e, w in enumerate(_head_pair(wqb_v, j, dm, nh)):
            qb_s[2 * j + e] = _dot(xb, w)

    w_copy("wuk").wait()

    for j in range(nh // 2):
        for e, w in enumerate(_head_pair(wuk_v, j, dc, nh)):
            h = 2 * j + e
            r = _dot_nt(qb_s[h].astype(_BF16), w)
            for c in range(ncc):
                lat_s[c, h * _ROWS:(h + 1) * _ROWS, :] = r[:, c * 128:(c + 1) * 128]
    for b in range(nb):
        rows = pl.ds(b, nh, stride=_ROWS)
        bat_s[b] = jnp.concatenate([lat_s[c, rows, :] for c in range(ncc)], axis=1)

    def latent_attention(b, carry):
        c_copy(b).wait()
        q = bat_s[b].astype(_BF16)

        def scores(t, m):
            keys = pl.ds(pl.multiple_of(t * _KC, _KC), _KC)
            s = _dot_nt(q, c_v[b, keys, :]) * scale
            sc_s[t] = s
            return jnp.maximum(m, s)

        m = lax.fori_loop(0, sk // _KC, scores, jnp.full((nh, _KC), -jnp.inf, _F32))
        m = jnp.max(m, axis=1, keepdims=True)

        def context(t, lo):
            l, o = lo
            keys = pl.ds(pl.multiple_of(t * _KC, _KC), _KC)
            p = jnp.exp(sc_s[t] - m)
            return l + p, o + _dot(p.astype(_BF16), c_v[b, keys, :])

        l, o = lax.fori_loop(0, sk // _KC, context,
                             (jnp.zeros((nh, _KC), _F32), jnp.zeros((nh, dc), _F32)))
        bat_s[b] = o / jnp.sum(l, axis=1, keepdims=True)
        return carry

    lax.fori_loop(0, nb, latent_attention, 0)
    for b in range(nb):
        rows = pl.ds(b, nh, stride=_ROWS)
        for c in range(ncc):
            lat_s[c, rows, :] = bat_s[b, :, c * 128:(c + 1) * 128]

    w_copy("wuv").wait()

    for j in range(nh // 2):
        for e, w in enumerate(_head_pair(wuv_v, j, dc, nh)):
            h = 2 * j + e
            rows = pl.ds(h * _ROWS, _ROWS)
            lat = jnp.concatenate([lat_s[c, rows, :] for c in range(ncc)], axis=1)
            qb_s[h] = _dot(lat.astype(_BF16), w)

    w_copy("wob").wait()

    def out_pair(j, acc):
        for e in range(2):
            h = 2 * j + e
            acc = acc + _dot_nt(qb_s[h].astype(_BF16), wob_v[h])
        return acc

    out_b = lax.fori_loop(0, nh // 2, out_pair, jnp.zeros((_ROWS, dm), _F32))
    out_ref[:, dm:] = out_b[:nb].astype(out_ref.dtype)

    w_copy("xa").wait()
    w_copy("wqa").wait()
    xa = _pad_rows(xa_v[...])

    def q_group(g, carry):
        cols = pl.ds(pl.multiple_of(g * 4 * dh, 4 * dh), 4 * dh)
        q = _dot(xa, wqa_v[:, cols])
        for e in range(4):
            qa_s[4 * g + e] = q[:, e * dh:(e + 1) * dh]
        return carry

    lax.fori_loop(0, nh // 4, q_group, 0)

    w_copy("woa").wait()
    o_s[...] = jnp.zeros_like(o_s)
    acc_s[...] = jnp.zeros_like(acc_s)
    row = lax.broadcasted_iota(jnp.int32, (_ROWS, dh), 0)

    def head(i, carry):
        h = i // nb
        b = i % nb
        slot = i % _RING
        more = i + _RING < nsteps

        k_copy(i).wait()
        s = _dot_nt(qa_s[h].astype(_BF16), kbuf[slot]) * scale

        @pl.when(more)
        def _():
            k_copy(i + _RING).start()

        p = jnp.exp(s - jnp.max(s, axis=1, keepdims=True))
        l = jnp.sum(p, axis=1, keepdims=True)

        v_copy(i).wait()
        o = _dot(p.astype(_BF16), vbuf[slot]) / l

        @pl.when(more)
        def _():
            v_copy(i + _RING).start(priority=1)

        o = jnp.where(row == b, o, o_s[...])
        o_s[...] = o

        @pl.when(b == nb - 1)
        def _():
            cols = pl.ds(pl.multiple_of(h * dh, dh), dh)
            acc_s[...] += _dot_nt(o.astype(_BF16), woa_v[:, cols])

        return carry

    lax.fori_loop(0, nsteps, head, 0)
    out_ref[:, :dm] = acc_s[:nb, :].astype(out_ref.dtype)


@jax.jit
def pallas_concat_heads__mha_block_cached__compressed_kv_cla__decode_kernel(
    A_x: jax.Array,
    A_k_cache: jax.Array,
    A_v_cache: jax.Array,
    A_wq: jax.Array,
    A_wo: jax.Array,
    B_x: jax.Array,
    B_c_kv: jax.Array,
    B_w_q: jax.Array,
    B_w_uk: jax.Array,
    B_w_uv: jax.Array,
    B_w_o: jax.Array,
):
    nb, sq, dm = A_x.shape
    _, nh, sk, dh = A_k_cache.shape
    dc = B_c_kv.shape[2]
    assert sq == 1 and nb <= _ROWS

    operands = (
        A_x.reshape(nb, dm), A_k_cache, A_v_cache, A_wq, A_wo.T,
        B_x.reshape(nb, dm), B_c_kv,
        B_w_q.reshape(dm * nh, dh), B_w_uk.reshape(dc * nh, dh), B_w_uv.reshape(dc * nh, dh),
        B_w_o.transpose(0, 2, 1),
    )
    vmem = functools.partial(pltpu.VMEM, dtype=_BF16)
    out = pl.pallas_call(
        _kernel,
        in_specs=[pl.BlockSpec(memory_space=pl.ANY)] * len(operands),
        out_specs=pl.BlockSpec(memory_space=pltpu.VMEM),
        out_shape=jax.ShapeDtypeStruct((nb, 2 * dm), A_x.dtype),
        scratch_shapes=[
            vmem((nb, dm)), vmem((nb, dm)),
            vmem((_RING, sk, dh)), vmem((_RING, sk, dh)),
            vmem((dm, nh * dh)), vmem((dm, nh * dh)),
            vmem((nb, sk, dc)),
            vmem((dm * nh, dh)), vmem((dc * nh, dh)), vmem((dc * nh, dh)),
            vmem((nh, dm, dh)),
            pltpu.VMEM((nh, _ROWS, dh), _F32),
            pltpu.VMEM((nh, _ROWS, dh), _F32),
            pltpu.VMEM((dc // 128, nh * _ROWS, 128), _F32),
            pltpu.VMEM((nb, nh, dc), _F32),
            pltpu.VMEM((sk // _KC, nh, _KC), _F32),
            pltpu.VMEM((_ROWS, dh), _F32),
            pltpu.VMEM((_ROWS, dm), _F32),
            pltpu.SemaphoreType.DMA((_RING,)),
            pltpu.SemaphoreType.DMA((_RING,)),
            pltpu.SemaphoreType.DMA((nb,)),
            pltpu.SemaphoreType.DMA((8,)),
        ],
        compiler_params=pltpu.CompilerParams(vmem_limit_bytes=100 * 1024 * 1024),
        name="mha_cla_decode",
    )(*operands)
    return out.reshape(nb, sq, 2 * dm)
```

```python
import functools

import jax
import jax.numpy as jnp
from jax import lax
import jax.experimental.pallas as pl
import jax.experimental.pallas.tpu as pltpu

_F32 = jnp.float32
_BF16 = jnp.bfloat16
_ROWS = 8
_RING = 4
_KC = 512


def _dot(a, b):
    return lax.dot_general(a, b, (((1,), (0,)), ((), ())), preferred_element_type=_F32)


def _dot_nt(a, b):
    return lax.dot_general(a, b, (((1,), (1,)), ((), ())), preferred_element_type=_F32)


def _head_pair(w_ref, j, rows, heads):
    w = w_ref.bitcast(jnp.uint32)[pl.ds(j, rows, stride=heads // 2), :]
    lo = lax.bitcast_convert_type(w << 16, _F32).astype(_BF16)
    hi = lax.bitcast_convert_type((w >> 16) << 16, _F32).astype(_BF16)
    return lo, hi


def _pad_rows(x):
    x = x.astype(_F32)
    pad = jnp.zeros((_ROWS - x.shape[0], x.shape[1]), _F32)
    return jnp.concatenate([x, pad], axis=0).astype(_BF16)


def _kernel(xa_hbm, k_hbm, v_hbm, wqa_hbm, woa_hbm,
            xb_hbm, c_hbm, wqb_hbm, wuk_hbm, wuv_hbm, wob_hbm,
            out_ref,
            xa_v, xb_v, kbuf, vbuf, wqa_v, woa_v, c_v, wqb_v, wuk_v, wuv_v, wob_v,
            qa_s, qb_s, lat_s, bat_s, sc_s, o_s, acc_s,
            sem):
    nb, nh, sk, dh = k_hbm.shape
    dm = xa_hbm.shape[1]
    dc = c_hbm.shape[2]
    ncc = dc // 128
    nsteps = nb * nh
    scale = dh ** -0.5

    def k_copy(i):
        slot = i % _RING
        return pltpu.make_async_copy(k_hbm.at[i % nb, i // nb], kbuf.at[slot], sem.at[slot])

    def v_copy(i):
        slot = i % _RING
        return pltpu.make_async_copy(v_hbm.at[i % nb, i // nb], vbuf.at[slot], sem.at[_RING + slot])

    def c_copy(b):
        return pltpu.make_async_copy(c_hbm.at[b], c_v.at[b], sem.at[2 * _RING + b])

    whole = {
        "xa": (xa_hbm, xa_v, 0), "xb": (xb_hbm, xb_v, 1),
        "wqb": (wqb_hbm, wqb_v, 2), "wuk": (wuk_hbm, wuk_v, 3),
        "wuv": (wuv_hbm, wuv_v, 4), "wob": (wob_hbm, wob_v, 5),
        "wqa": (wqa_hbm, wqa_v, 6), "woa": (woa_hbm, woa_v, 7),
    }

    def w_copy(name):
        src, dst, s = whole[name]
        return pltpu.make_async_copy(src, dst, sem.at[2 * _RING + nb + s])

    w_copy("wqb").start()
    w_copy("xb").start(priority=1)
    w_copy("xa").start(priority=1)
    w_copy("wuk").start(priority=1)
    for b in range(nb):
        c_copy(b).start(priority=b % 2)
    w_copy("wuv").start()
    w_copy("wob").start(priority=1)
    w_copy("wqa").start()
    w_copy("woa").start(priority=1)
    for i in range(_RING):
        k_copy(i).start()
        v_copy(i).start(priority=1)

    w_copy("xb").wait()
    w_copy("wqb").wait()
    xb = _pad_rows(xb_v[...])

    for j in range(nh // 2):
        for e, w in enumerate(_head_pair(wqb_v, j, dm, nh)):
            qb_s[2 * j + e] = _dot(xb, w)

    w_copy("wuk").wait()

    for j in range(nh // 2):
        for e, w in enumerate(_head_pair(wuk_v, j, dc, nh)):
            h = 2 * j + e
            r = _dot_nt(qb_s[h].astype(_BF16), w)
            for c in range(ncc):
                lat_s[c, h * _ROWS:(h + 1) * _ROWS, :] = r[:, c * 128:(c + 1) * 128]
    for b in range(nb):
        rows = pl.ds(b, nh, stride=_ROWS)
        bat_s[b] = jnp.concatenate([lat_s[c, rows, :] for c in range(ncc)], axis=1)

    def latent_attention(b, carry):
        c_copy(b).wait()
        q = bat_s[b].astype(_BF16)

        def scores(t, m):
            keys = pl.ds(pl.multiple_of(t * _KC, _KC), _KC)
            s = _dot_nt(q, c_v[b, keys, :]) * scale
            sc_s[t] = s
            return jnp.maximum(m, s)

        m = lax.fori_loop(0, sk // _KC, scores, jnp.full((nh, _KC), -jnp.inf, _F32))
        m = jnp.max(m, axis=1, keepdims=True)

        def context(t, lo):
            l, o = lo
            keys = pl.ds(pl.multiple_of(t * _KC, _KC), _KC)
            p = jnp.exp(sc_s[t] - m)
            return l + p, o + _dot(p.astype(_BF16), c_v[b, keys, :])

        l, o = lax.fori_loop(0, sk // _KC, context,
                             (jnp.zeros((nh, _KC), _F32), jnp.zeros((nh, dc), _F32)))
        bat_s[b] = o / jnp.sum(l, axis=1, keepdims=True)
        return carry

    lax.fori_loop(0, nb, latent_attention, 0)
    for b in range(nb):
        rows = pl.ds(b, nh, stride=_ROWS)
        for c in range(ncc):
            lat_s[c, rows, :] = bat_s[b, :, c * 128:(c + 1) * 128]

    w_copy("wuv").wait()

    for j in range(nh // 2):
        for e, w in enumerate(_head_pair(wuv_v, j, dc, nh)):
            h = 2 * j + e
            rows = pl.ds(h * _ROWS, _ROWS)
            lat = jnp.concatenate([lat_s[c, rows, :] for c in range(ncc)], axis=1)
            qb_s[h] = _dot(lat.astype(_BF16), w)

    w_copy("wob").wait()

    def out_pair(j, acc):
        for e in range(2):
            h = 2 * j + e
            acc = acc + _dot_nt(qb_s[h].astype(_BF16), wob_v[h])
        return acc

    out_b = lax.fori_loop(0, nh // 2, out_pair, jnp.zeros((_ROWS, dm), _F32))
    out_ref[:, dm:] = out_b[:nb].astype(out_ref.dtype)

    w_copy("xa").wait()
    w_copy("wqa").wait()
    xa = _pad_rows(xa_v[...])

    def q_group(g, carry):
        cols = pl.ds(pl.multiple_of(g * 4 * dh, 4 * dh), 4 * dh)
        q = _dot(xa, wqa_v[:, cols])
        for e in range(4):
            qa_s[4 * g + e] = q[:, e * dh:(e + 1) * dh]
        return carry

    lax.fori_loop(0, nh // 4, q_group, 0)

    w_copy("woa").wait()
    o_s[...] = jnp.zeros_like(o_s)
    acc_s[...] = jnp.zeros_like(acc_s)
    row = lax.broadcasted_iota(jnp.int32, (_ROWS, dh), 0)

    def head(i, carry):
        h = i // nb
        b = i % nb
        slot = i % _RING
        more = i + _RING < nsteps

        k_copy(i).wait()
        s = _dot_nt(qa_s[h].astype(_BF16), kbuf[slot]) * scale

        @pl.when(more)
        def _():
            k_copy(i + _RING).start()

        p = jnp.exp(s - jnp.max(s, axis=1, keepdims=True))
        l = jnp.sum(p, axis=1, keepdims=True)

        v_copy(i).wait()
        o = _dot(p.astype(_BF16), vbuf[slot]) / l

        @pl.when(more)
        def _():
            v_copy(i + _RING).start(priority=1)

        o = jnp.where(row == b, o, o_s[...])
        o_s[...] = o

        @pl.when(b == nb - 1)
        def _():
            cols = pl.ds(pl.multiple_of(h * dh, dh), dh)
            acc_s[...] += _dot_nt(o.astype(_BF16), woa_v[:, cols])

        return carry

    lax.fori_loop(0, nsteps, head, 0)
    out_ref[:, :dm] = acc_s[:nb, :].astype(out_ref.dtype)


@jax.jit
def pallas_concat_heads__mha_block_cached__compressed_kv_cla__decode_kernel(
    A_x: jax.Array,
    A_k_cache: jax.Array,
    A_v_cache: jax.Array,
    A_wq: jax.Array,
    A_wo: jax.Array,
    B_x: jax.Array,
    B_c_kv: jax.Array,
    B_w_q: jax.Array,
    B_w_uk: jax.Array,
    B_w_uv: jax.Array,
    B_w_o: jax.Array,
):
    nb, sq, dm = A_x.shape
    _, nh, sk, dh = A_k_cache.shape
    dc = B_c_kv.shape[2]
    assert sq == 1 and nb <= _ROWS

    operands = (
        A_x.reshape(nb, dm), A_k_cache, A_v_cache, A_wq, A_wo.T,
        B_x.reshape(nb, dm), B_c_kv,
        B_w_q.reshape(dm * nh, dh), B_w_uk.reshape(dc * nh, dh), B_w_uv.reshape(dc * nh, dh),
        B_w_o.transpose(0, 2, 1),
    )
    vmem = functools.partial(pltpu.VMEM, dtype=_BF16)
    out = pl.pallas_call(
        _kernel,
        in_specs=[pl.BlockSpec(memory_space=pl.ANY)] * len(operands),
        out_specs=pl.BlockSpec(memory_space=pltpu.VMEM),
        out_shape=jax.ShapeDtypeStruct((nb, 2 * dm), A_x.dtype),
        scratch_shapes=[
            vmem((nb, dm)), vmem((nb, dm)),
            vmem((_RING, sk, dh)), vmem((_RING, sk, dh)),
            vmem((dm, nh * dh)), vmem((dm, nh * dh)),
            vmem((nb, sk, dc)),
            vmem((dm * nh, dh)), vmem((dc * nh, dh)), vmem((dc * nh, dh)),
            vmem((nh, dm, dh)),
            pltpu.VMEM((nh, _ROWS, dh), _F32),
            pltpu.VMEM((nh, _ROWS, dh), _F32),
            pltpu.VMEM((dc // 128, nh * _ROWS, 128), _F32),
            pltpu.VMEM((nb, nh, dc), _F32),
            pltpu.VMEM((sk // _KC, nh, _KC), _F32),
            pltpu.VMEM((_ROWS, dh), _F32),
            pltpu.VMEM((_ROWS, dm), _F32),
            pltpu.SemaphoreType.DMA((2 * _RING + nb + 8,)),
        ],
        compiler_params=pltpu.CompilerParams(vmem_limit_bytes=100 * 1024 * 1024),
        name="mha_cla_decode",
    )(*operands)
    return out.reshape(nb, sq, 2 * dm)
```

```python
import functools

import jax
import jax.numpy as jnp
from jax import lax
import jax.experimental.pallas as pl
import jax.experimental.pallas.tpu as pltpu

_F32 = jnp.float32
_BF16 = jnp.bfloat16
_ROWS = 8
_RING = 4
_AHEAD = 3
_KC = 1024
_KVROWS = 128
_UNROLL = 4
_PARAMS = dict()


def _dot(a, b):
    return lax.dot_general(a, b, (((1,), (0,)), ((), ())), preferred_element_type=_F32)


def _dot_nt(a, b):
    return lax.dot_general(a, b, (((1,), (1,)), ((), ())), preferred_element_type=_F32)


def _eight_heads(w_ref, g, rows, heads):
    stride = heads // 2
    words = w_ref.bitcast(jnp.uint32).at[pl.ds(pl.multiple_of(4 * g, 4), (rows - 1) * stride + 4)]
    for j in range(4):
        w = words[pl.ds(j, rows, stride=stride), :]
        yield lax.bitcast_convert_type(w << 16, _F32).astype(_BF16)
        yield lax.bitcast_convert_type((w >> 16) << 16, _F32).astype(_BF16)


def _pad_rows(x):
    x = x.astype(_F32)
    pad = jnp.zeros((_ROWS - x.shape[0], x.shape[1]), _F32)
    return jnp.concatenate([x, pad], axis=0).astype(_BF16)


def _row_piece(src, dst, sem, pieces):
    rows = src.shape[0] // pieces

    def piece(j):
        sl = pl.ds(pl.multiple_of(j * rows, rows), rows)
        return pltpu.make_async_copy(src.at[sl], dst.at[sl], sem)
    return piece


def _wide_piece(src, dst, sem):
    cols = src.shape[1] // 2

    def piece(j):
        sl = (pl.ds(pl.multiple_of((j >> 1) * 8, 8), 8),
              pl.ds(pl.multiple_of((j & 1) * cols, cols), cols))
        return pltpu.make_async_copy(src.at[sl], dst.at[sl], sem)
    return piece


def _request(hi, lo, first, count):
    unroll = _UNROLL if count % _UNROLL == 0 else 2

    def body(t, carry):
        for u in range(unroll):
            j = first + t * unroll + u
            hi(j).start(priority=0)
            lo(j).start(priority=1)
        return carry
    lax.fori_loop(0, count // unroll, body, 0)


def _arrived(buf, sem):
    pltpu.make_async_copy(buf, buf, sem).wait()


def _kernel(xa_hbm, k_hbm, v_hbm, wqa_hbm, woa_hbm,
            xb_hbm, c_hbm, wqb_hbm, wuk_hbm, wuv_hbm, wob_hbm,
            out_ref,
            xa_v, xb_v, kbuf, vbuf, wqa_v, woa_v, c_v, wqb_v, wuk_v, wuv_v, wob_v,
            qa_s, qb_s, lat_s, bat_s, sc_s, o_s, acc_s,
            sem):
    nb, nh, sk, dh = k_hbm.shape
    dm = xa_hbm.shape[1]
    dc = c_hbm.shape[2]
    ncc = dc // 128
    nsteps = nb * nh
    scale = dh ** -0.5

    c_sem = lambda b: sem.at[b]
    wqb_sem, wuk_sem, xb_sem, xa_sem = sem.at[4], sem.at[5], sem.at[6], sem.at[7]
    wuv_sem, wob_sem = sem.at[4], sem.at[5]
    wqa_sem, woa_sem = sem.at[3], sem.at[7]

    wqb = _row_piece(wqb_hbm, wqb_v, wqb_sem, 128)
    wuk = _row_piece(wuk_hbm, wuk_v, wuk_sem, 128)
    wuv = _row_piece(wuv_hbm, wuv_v, wuv_sem, 128)
    wob = _row_piece(wob_hbm, wob_v, wob_sem, 128)
    lat = [_row_piece(c_hbm.at[b], c_v.at[b], c_sem(b), 128) for b in range(nb)]
    wqa = _wide_piece(wqa_hbm, wqa_v, wqa_sem)
    woa = _wide_piece(woa_hbm, woa_v, woa_sem)
    kv_pieces = sk // _KVROWS

    def request_head(i, first=0, count=kv_pieces):
        b, h, slot = i % nb, i // nb, i % _RING
        _request(_row_piece(k_hbm.at[b, h], kbuf.at[slot], sem.at[slot], kv_pieces),
                 _row_piece(v_hbm.at[b, h], vbuf.at[slot], sem.at[_RING + slot], kv_pieces),
                 first, count)

    _request(wqb, wuk, 0, 128)
    pltpu.make_async_copy(xb_hbm, xb_v, xb_sem).start()
    pltpu.make_async_copy(xa_hbm, xa_v, xa_sem).start()
    _request(lat[0], lat[1], 0, 32)

    _arrived(xb_v, xb_sem)
    _arrived(xa_v, xa_sem)
    _arrived(wqb_v, wqb_sem)
    xb = _pad_rows(xb_v[...])

    def q_group(g, carry):
        for e, w in enumerate(_eight_heads(wqb_v, g, dm, nh)):
            qb_s[8 * g + e] = _dot(xb, w)
        _request(lat[0], lat[1], 32 + 12 * g, 12)
        return carry

    lax.fori_loop(0, nh // 8, q_group, 0)

    _arrived(wuk_v, wuk_sem)

    def absorb_group(g, carry):
        for e, w in enumerate(_eight_heads(wuk_v, g, dc, nh)):
            h = 8 * g + e
            r = _dot_nt(qb_s[h].astype(_BF16), w)
            rows = pl.ds(pl.multiple_of(h * _ROWS, _ROWS), _ROWS)
            for c in range(ncc):
                lat_s[c, rows, :] = r[:, c * 128:(c + 1) * 128]
        _request(lat[0], lat[1], 80 + 12 * g, 12)
        return carry

    lax.fori_loop(0, nh // 8, absorb_group, 0)
    for b in range(nb):
        rows = pl.ds(b, nh, stride=_ROWS)
        bat_s[b] = jnp.concatenate([lat_s[c, rows, :] for c in range(ncc)], axis=1)

    nkc = sk // _KC
    per = 48 // (2 * nkc)

    def latent_attention(b, carry):
        def request(first, count):
            @pl.when(b < 2)
            def _():
                _request(lat[2], lat[3], first, count)

            @pl.when(b >= 2)
            def _():
                _request(wuv, wob, first, count)

        @pl.when(b % 2 == 0)
        def _():
            request(0, 32)

        base = 32 + 48 * (b % 2)
        _arrived(c_v.at[b], c_sem(b))
        q = bat_s[b].astype(_BF16)

        def scores(t, m):
            keys = pl.ds(pl.multiple_of(t * _KC, _KC), _KC)
            s = _dot_nt(q, c_v[b, keys, :]) * scale
            sc_s[t] = s
            for c in range(_KC // 128):
                m = jnp.maximum(m, s[:, c * 128:(c + 1) * 128])
            request(base + per * t, per)
            return m

        m = lax.fori_loop(0, nkc, scores, jnp.full((nh, 128), -jnp.inf, _F32))
        m = jnp.max(m, axis=1, keepdims=True)

        def context(t, lo):
            l, o = lo
            keys = pl.ds(pl.multiple_of(t * _KC, _KC), _KC)
            p = jnp.exp(sc_s[t] - m)
            for c in range(_KC // 128):
                l = l + p[:, c * 128:(c + 1) * 128]
            o = o + _dot(p.astype(_BF16), c_v[b, keys, :])
            request(base + per * (nkc + t), per)
            return l, o

        l, o = lax.fori_loop(0, nkc, context,
                             (jnp.zeros((nh, 128), _F32), jnp.zeros((nh, dc), _F32)))
        bat_s[b] = o / jnp.sum(l, axis=1, keepdims=True)
        return carry

    lax.fori_loop(0, nb, latent_attention, 0)
    for b in range(nb):
        rows = pl.ds(b, nh, stride=_ROWS)
        for c in range(ncc):
            lat_s[c, rows, :] = bat_s[b, :, c * 128:(c + 1) * 128]

    _request(wqa, woa, 0, 32)
    _arrived(wuv_v, wuv_sem)

    def value_group(g, carry):
        for e, w in enumerate(_eight_heads(wuv_v, g, dc, nh)):
            h = 8 * g + e
            rows = pl.ds(pl.multiple_of(h * _ROWS, _ROWS), _ROWS)
            x = jnp.concatenate([lat_s[c, rows, :] for c in range(ncc)], axis=1)
            qb_s[h] = _dot(x.astype(_BF16), w)
        _request(wqa, woa, 32 + 12 * g, 12)
        return carry

    lax.fori_loop(0, nh // 8, value_group, 0)
    _arrived(wob_v, wob_sem)

    def out_group(g, acc):
        for e in range(4):
            h = 4 * g + e
            rows = pl.ds(pl.multiple_of(h * dm, dm), dm)
            acc = acc + _dot_nt(qb_s[h].astype(_BF16), wob_v[rows, :])
        _request(wqa, woa, 80 + 8 * g, 8)
        return acc

    out_b = lax.fori_loop(0, nh // 4, out_group, jnp.zeros((_ROWS, dm), _F32))
    out_ref[:, dm:] = out_b[:nb].astype(out_ref.dtype)

    request_head(0)
    _arrived(wqa_v, wqa_sem)
    xa = _pad_rows(xa_v[...])

    def qa_group(g, carry):
        cols = pl.ds(pl.multiple_of(g * 4 * dh, 4 * dh), 4 * dh)
        q = _dot(xa, wqa_v[:, cols])
        for e in range(4):
            qa_s[4 * g + e] = q[:, e * dh:(e + 1) * dh]
        request_head(1, g * (kv_pieces // 8), kv_pieces // 8)
        return carry

    lax.fori_loop(0, nh // 4, qa_group, 0)
    for i in range(2, _AHEAD):
        request_head(i)

    _arrived(woa_v, woa_sem)
    o_s[...] = jnp.zeros_like(o_s)
    acc_s[...] = jnp.zeros_like(acc_s)
    row = lax.broadcasted_iota(jnp.int32, (_ROWS, dh), 0)

    def head(i, carry):
        h = i // nb
        b = i % nb
        slot = i % _RING

        _arrived(kbuf.at[slot], sem.at[slot])
        s = _dot_nt(qa_s[h].astype(_BF16), kbuf[slot]) * scale
        p = jnp.exp(s - jnp.max(s, axis=1, keepdims=True))
        l = jnp.sum(p, axis=1, keepdims=True)
        p = p.astype(_BF16)

        _arrived(vbuf.at[slot], sem.at[_RING + slot])
        o = _dot(p, vbuf[slot]) / l
        o = jnp.where(row == b, o, o_s[...])
        o_s[...] = o

        @pl.when(b == nb - 1)
        def _():
            cols = pl.ds(pl.multiple_of(h * dh, dh), dh)
            acc_s[...] += _dot_nt(o.astype(_BF16), woa_v[:, cols])

        @pl.when(i + _AHEAD < nsteps)
        def _():
            request_head(i + _AHEAD)

        return carry

    lax.fori_loop(0, nsteps, head, 0)
    out_ref[:, :dm] = acc_s[:nb, :].astype(out_ref.dtype)


@jax.jit
def pallas_concat_heads__mha_block_cached__compressed_kv_cla__decode_kernel(
    A_x: jax.Array,
    A_k_cache: jax.Array,
    A_v_cache: jax.Array,
    A_wq: jax.Array,
    A_wo: jax.Array,
    B_x: jax.Array,
    B_c_kv: jax.Array,
    B_w_q: jax.Array,
    B_w_uk: jax.Array,
    B_w_uv: jax.Array,
    B_w_o: jax.Array,
):
    nb, sq, dm = A_x.shape
    _, nh, sk, dh = A_k_cache.shape
    dc = B_c_kv.shape[2]
    assert sq == 1 and nb <= _ROWS

    operands = (
        A_x.reshape(nb, dm), A_k_cache, A_v_cache, A_wq, A_wo.T,
        B_x.reshape(nb, dm), B_c_kv,
        B_w_q.reshape(dm * nh, dh), B_w_uk.reshape(dc * nh, dh), B_w_uv.reshape(dc * nh, dh),
        B_w_o.transpose(0, 2, 1).reshape(nh * dm, dh),
    )
    vmem = functools.partial(pltpu.VMEM, dtype=_BF16)
    out = pl.pallas_call(
        _kernel,
        in_specs=[pl.BlockSpec(memory_space=pl.ANY)] * len(operands),
        out_specs=pl.BlockSpec(memory_space=pltpu.VMEM),
        out_shape=jax.ShapeDtypeStruct((nb, 2 * dm), A_x.dtype),
        scratch_shapes=[
            vmem((nb, dm)), vmem((nb, dm)),
            vmem((_RING, sk, dh)), vmem((_RING, sk, dh)),
            vmem((dm, nh * dh)), vmem((dm, nh * dh)),
            vmem((nb, sk, dc)),
            vmem((dm * nh, dh)), vmem((dc * nh, dh)), vmem((dc * nh, dh)),
            vmem((nh * dm, dh)),
            pltpu.VMEM((nh, _ROWS, dh), _F32),
            pltpu.VMEM((nh, _ROWS, dh), _F32),
            pltpu.VMEM((dc // 128, nh * _ROWS, 128), _F32),
            pltpu.VMEM((nb, nh, dc), _F32),
            pltpu.VMEM((sk // _KC, nh, _KC), _F32),
            pltpu.VMEM((_ROWS, dh), _F32),
            pltpu.VMEM((_ROWS, dm), _F32),
            pltpu.SemaphoreType.DMA((2 * _RING,)),
        ],
        compiler_params=pltpu.CompilerParams(vmem_limit_bytes=100 * 1024 * 1024, **_PARAMS),
        name="mha_cla_decode",
    )(*operands)
    return out.reshape(nb, sq, 2 * dm)
```

```python
import functools

import jax
import jax.numpy as jnp
from jax import lax
import jax.experimental.pallas as pl
import jax.experimental.pallas.tpu as pltpu

_F32 = jnp.float32
_BF16 = jnp.bfloat16
_ROWS = 8
_RING = 4
_KB = 512
_KC = 1024
_SEG = 8192
_PARAMS = dict()


def _dot(a, b):
    return lax.dot_general(a, b, (((1,), (0,)), ((), ())), preferred_element_type=_F32)


def _dot_nt(a, b):
    return lax.dot_general(a, b, (((1,), (1,)), ((), ())), preferred_element_type=_F32)


def _span(start, size):
    return pl.ds(pl.multiple_of(start, size), size)


def _eight_heads(w_ref, g, heads):
    stride = heads // 2
    rows = w_ref.shape[1] // heads
    words = w_ref.bitcast(jnp.uint32).at[:, pl.ds(pl.multiple_of(4 * g, 4), (rows - 1) * stride + 4)]
    for j in range(4):
        w = jnp.concatenate([words[i, pl.ds(j, rows, stride=stride), :] for i in range(2)], axis=0)
        yield lax.bitcast_convert_type(w << 16, _F32).astype(_BF16)
        yield lax.bitcast_convert_type((w >> 16) << 16, _F32).astype(_BF16)


def _pad_rows(x):
    x = x.astype(_F32)
    pad = jnp.zeros((_ROWS - x.shape[0], x.shape[1]), _F32)
    return jnp.concatenate([x, pad], axis=0).astype(_BF16)


def _halves(src, dst, sem):
    _, rows, cols = src.shape
    quarter = rows * cols // _SEG // 4

    def piece(t, u):
        s = u * quarter + t
        if cols * _ROWS <= _SEG:
            idx = (slice(None), _span(s * (_SEG // cols), _SEG // cols))
        else:
            width = _SEG // _ROWS
            n = cols // width
            idx = (slice(None), _span(s // n * _ROWS, _ROWS), _span(s % n * width, width))
        return pltpu.make_async_copy(src.at[idx], dst.at[idx], sem)
    return piece


def _request(hi, lo, first, rounds):
    def body(t, carry):
        for u in range(4):
            hi(first + t, u).start(priority=0)
            lo(first + t, u).start(priority=1)
        return carry
    lax.fori_loop(0, rounds, body, 0)


def _arrived(buf, sem):
    pltpu.make_async_copy(buf, buf, sem).wait()


def _kernel(xa_hbm, k_hbm, v_hbm, wqa_hbm, woa_hbm,
            xb_hbm, c_hbm, wqb_hbm, wuk_hbm, wuv_hbm, wob_hbm,
            out_ref,
            xa_v, xb_v, kbuf, vbuf, wqa_v, woa_v, c_v, wqb_v, wuk_v, wuv_v, wob_v,
            hd_s, qt_s, qb_s, lat_s, bat_s, sc_s,
            sem):
    nb, nh, sk, dh = k_hbm.shape
    dm = xa_hbm.shape[1]
    dc = c_hbm.shape[3]
    ncc = dc // 128
    nkb = sk // _KB
    ngrp = nh // _ROWS
    nsteps = nb * ngrp * nkb
    scale = dh ** -0.5

    wqb_sem, wqa_sem, wuk_sem, wuv_sem, x_sem = (sem.at[n] for n in (0, 1, 2, 8, 3))
    c_sem = lambda b: sem.at[4 + b]
    wob_sem = sem.at[4]
    woa_sem = [sem.at[4 + n] for n in range(3)]

    wqb, wqa = _halves(wqb_hbm, wqb_v, wqb_sem), _halves(wqa_hbm, wqa_v, wqa_sem)
    wuk, wuv = _halves(wuk_hbm, wuk_v, wuk_sem), _halves(wuv_hbm, wuv_v, wuv_sem)
    lat = [_halves(c_hbm.at[b], c_v.at[b], c_sem(b)) for b in range(nb)]
    wob = [_halves(wob_hbm.at[n], wob_v.at[n], wob_sem) for n in range(2)]

    def request_step(i, first=0, rounds=_KB * dh // _SEG):
        grp, kb, slot = i // nkb, i % nkb, i % _RING
        b, g = grp // ngrp, grp % ngrp
        n = _SEG // dh

        def cache(src, dst):
            def piece(t, u):
                return pltpu.make_async_copy(
                    src.at[b, pl.ds(g * _ROWS + 2 * u, 2), _span(kb * _KB + t * n, n)],
                    dst.at[slot, pl.ds(2 * u, 2), _span(t * n, n)], sem.at[slot])
            return piece
        _request(cache(k_hbm, kbuf), cache(v_hbm, vbuf), first, rounds)

    def woa(n):
        width = _SEG // _ROWS

        def piece(t, u):
            s = 2 * t + u // 2
            idx = (pl.ds(4 * n + 2 * (u % 2), 2), _span(s // 4 * _ROWS, _ROWS), _span(s % 4 * width, width))
            return pltpu.make_async_copy(woa_hbm.at[idx], woa_v.at[idx], woa_sem[n])
        return piece

    _request(wqb, wqa, 0, 36)
    pltpu.make_async_copy(xb_hbm, xb_v, x_sem).start()
    pltpu.make_async_copy(xa_hbm, xa_v, x_sem).start()
    _request(wuk, wuv, 0, 8)

    _arrived(xb_v, x_sem)
    _arrived(xa_v, x_sem)
    _arrived(wqb_v, wqb_sem)
    xb = _pad_rows(xb_v[...])

    def qb_group(g, carry):
        for e, w in enumerate(_eight_heads(wqb_v, g, nh)):
            qb_s[8 * g + e] = _dot(xb, w)
        _request(wuk, wuv, 8 + 4 * g, 4)
        return carry

    lax.fori_loop(0, ngrp, qb_group, 0)
    _arrived(wqa_v, wqa_sem)
    xa = _pad_rows(xa_v[...])

    def qa_group(g, carry):
        q = _dot(xa, wqa_v[:, :, _span(g * _ROWS * dh, _ROWS * dh)].reshape(dm, _ROWS * dh))
        for e in range(_ROWS):
            hd_s[_span((g * _ROWS + e) * _ROWS, _ROWS), :] = q[:, e * dh:(e + 1) * dh]
        _request(wuk, wuv, 24 + 2 * g, 2)
        return carry

    lax.fori_loop(0, ngrp, qa_group, 0)
    for b in range(nb):
        qt_s[b * nh:(b + 1) * nh, :] = hd_s[pl.ds(b, nh, stride=_ROWS), :]

    _request(lat[0], lat[1], 0, 16)
    _arrived(wuk_v, wuk_sem)

    def absorb_group(g, carry):
        for e, w in enumerate(_eight_heads(wuk_v, g, nh)):
            h = 8 * g + e
            r = _dot_nt(qb_s[h].astype(_BF16), w)
            for c in range(ncc):
                lat_s[c, _span(h * _ROWS, _ROWS), :] = r[:, c * 128:(c + 1) * 128]
        _request(lat[0], lat[1], 16 + 4 * g, 4)
        return carry

    lax.fori_loop(0, ngrp, absorb_group, 0)
    for b in range(nb):
        rows = pl.ds(b, nh, stride=_ROWS)
        bat_s[b] = jnp.concatenate([lat_s[c, rows, :] for c in range(ncc)], axis=1)

    nkc = sk // _KC
    per_half = nkc // 2

    def latent_attention(b, carry):
        def request(first, rounds):
            @pl.when(b < 2)
            def _():
                _request(lat[2], lat[3], 8 + 12 * b + first, rounds)

            @pl.when(b == 2)
            def _():
                _request(wob[0], wob[1], 6 + first, rounds)

            @pl.when((b == 3) & (first < 8))
            def _():
                request_step(0, first, rounds)

            @pl.when((b == 3) & (first >= 8))
            def _():
                request_step(1, first - 8, rounds)

        @pl.when(b == 0)
        def _():
            _request(lat[2], lat[3], 0, 8)

        @pl.when(b == 2)
        def _():
            _request(wob[0], wob[1], 0, 6)

        _arrived(c_v.at[b], c_sem(b))
        q = bat_s[b].astype(_BF16)

        def latents(t):
            return c_v[b, t // per_half, _span(t % per_half * _KC, _KC), :]

        def scores(t, m):
            s = _dot_nt(q, latents(t)) * scale
            sc_s[t] = s
            for c in range(_KC // 128):
                m = jnp.maximum(m, s[:, c * 128:(c + 1) * 128])
            request(2 * t, 2)
            return m

        m = lax.fori_loop(0, nkc, scores, jnp.full((nh, 128), -jnp.inf, _F32))
        m = jnp.max(m, axis=1, keepdims=True)

        def context(t, lo):
            l, o = lo
            p = jnp.exp(sc_s[t] - m)
            for c in range(_KC // 128):
                l = l + p[:, c * 128:(c + 1) * 128]
            o = o + _dot(p.astype(_BF16), latents(t))
            request(2 * nkc + t, 1)
            return l, o

        l, o = lax.fori_loop(0, nkc, context,
                             (jnp.zeros((nh, 128), _F32), jnp.zeros((nh, dc), _F32)))
        bat_s[b] = o / jnp.sum(l, axis=1, keepdims=True)
        return carry

    lax.fori_loop(0, nb, latent_attention, 0)
    for b in range(nb):
        rows = pl.ds(b, nh, stride=_ROWS)
        for c in range(ncc):
            lat_s[c, rows, :] = bat_s[b, :, c * 128:(c + 1) * 128]

    request_step(1, 4, 4)
    _arrived(wuv_v, wuv_sem)

    def value_group(g, carry):
        for e, w in enumerate(_eight_heads(wuv_v, g, nh)):
            h = 8 * g + e
            x = jnp.concatenate([lat_s[c, _span(h * _ROWS, _ROWS), :] for c in range(ncc)], axis=1)
            qb_s[h] = _dot(x.astype(_BF16), w)
        request_step(2, 2 * g, 2)
        return carry

    lax.fori_loop(0, ngrp, value_group, 0)
    _arrived(wob_v, wob_sem)

    def out_group(g, acc):
        for e in range(_ROWS):
            w = wob_v[g // 2, g % 2, e * dm:(e + 1) * dm, :]
            acc = acc + _dot_nt(qb_s[_ROWS * g + e].astype(_BF16), w)
        request_step(3, 2 * g, 2)
        return acc

    out_b = lax.fori_loop(0, ngrp, out_group, jnp.zeros((_ROWS, dm), _F32))
    out_ref[:, dm:] = out_b[:nb].astype(out_ref.dtype)

    row = lax.broadcasted_iota(jnp.int32, (_ROWS, _KB), 0)

    def group(grp, carry):
        q = qt_s[_span(grp * _ROWS, _ROWS), :].astype(_BF16)

        def step(kb, state):
            m, l, acc = state
            i = grp * nkb + kb
            slot = i % _RING
            _arrived(kbuf.at[slot], sem.at[slot])
            _arrived(vbuf.at[slot], sem.at[slot])
            full = _dot_nt(q, kbuf[slot].reshape(_ROWS * _KB, dh))
            s = full[:, :_KB]
            for e in range(1, _ROWS):
                s = jnp.where(row == e, full[:, e * _KB:(e + 1) * _KB], s)
            s = s * scale
            m_new = jnp.maximum(m, jnp.max(s, axis=1, keepdims=True))
            alpha = jnp.exp(m - m_new)
            p = jnp.exp(s - m_new)
            l = alpha * l + jnp.sum(p, axis=1, keepdims=True)
            spread = jnp.concatenate([jnp.where(row == e, p, 0.0) for e in range(_ROWS)], axis=1)
            acc = alpha * acc + _dot(spread.astype(_BF16), vbuf[slot].reshape(_ROWS * _KB, dh))

            @pl.when(i + _RING < nsteps)
            def _():
                request_step(i + _RING)

            @pl.when(i + _RING >= nsteps)
            def _():
                _request(woa(0), woa(1), (i + _RING - nsteps) * 4, 4)

            return m_new, l, acc

        _, l, acc = lax.fori_loop(
            0, nkb, step,
            (jnp.full((_ROWS, 1), -jnp.inf, _F32), jnp.zeros((_ROWS, 1), _F32),
             jnp.zeros((_ROWS, dh), _F32)))
        qt_s[_span(grp * _ROWS, _ROWS), :] = acc / l
        return carry

    lax.fori_loop(0, nb * ngrp, group, 0)
    pltpu.make_async_copy(woa_hbm.at[8], woa_v.at[8], woa_sem[2]).start(priority=1)

    for b in range(nb):
        hd_s[pl.ds(b, nh, stride=_ROWS), :] = qt_s[b * nh:(b + 1) * nh, :]
    o = jnp.concatenate([hd_s[h * _ROWS:(h + 1) * _ROWS, :] for h in range(nh)], axis=1)
    o = o.astype(_BF16)
    for n, (lo, hi) in enumerate(((0, 4), (4, 8), (8, 9))):
        _arrived(woa_v.at[lo:hi], woa_sem[n])
        w = woa_v[lo:hi].reshape((hi - lo) * 64, nh * dh)
        out_ref[:, lo * 64:hi * 64] = _dot_nt(o, w)[:nb].astype(out_ref.dtype)


@jax.jit
def pallas_concat_heads__mha_block_cached__compressed_kv_cla__decode_kernel(
    A_x: jax.Array,
    A_k_cache: jax.Array,
    A_v_cache: jax.Array,
    A_wq: jax.Array,
    A_wo: jax.Array,
    B_x: jax.Array,
    B_c_kv: jax.Array,
    B_w_q: jax.Array,
    B_w_uk: jax.Array,
    B_w_uv: jax.Array,
    B_w_o: jax.Array,
):
    nb, sq, dm = A_x.shape
    _, nh, sk, dh = A_k_cache.shape
    dc = B_c_kv.shape[2]
    assert (nb, sq, dm, nh, sk, dh, dc) == (4, 1, 576, 32, 4096, 128, 512)

    xa, xb = A_x.reshape(nb, dm), B_x.reshape(nb, dm)
    wqa = A_wq.reshape(2, dm // 2, nh * dh)
    woa = A_wo.T.reshape(dm // 64, 64, nh * dh)
    c = B_c_kv.reshape(nb, 2, sk // 2, dc)
    wqb = B_w_q.reshape(2, dm // 2 * nh, dh)
    wuk = B_w_uk.reshape(2, dc // 2 * nh, dh)
    wuv = B_w_uv.reshape(2, dc // 2 * nh, dh)
    wob = B_w_o.transpose(0, 2, 1).reshape(2, 2, nh // 4 * dm, dh)
    operands = (xa, A_k_cache, A_v_cache, wqa, woa, xb, c, wqb, wuk, wuv, wob)

    like = lambda a: pltpu.VMEM(a.shape, a.dtype)
    ring = pltpu.VMEM((_RING, _ROWS, _KB, dh), A_k_cache.dtype)
    out = pl.pallas_call(
        _kernel,
        in_specs=[pl.BlockSpec(memory_space=pl.ANY)] * len(operands),
        out_specs=pl.BlockSpec(memory_space=pltpu.VMEM),
        out_shape=jax.ShapeDtypeStruct((nb, 2 * dm), A_x.dtype),
        scratch_shapes=[
            like(xa), like(xb), ring, ring, like(wqa), like(woa),
            like(c), like(wqb), like(wuk), like(wuv), like(wob),
            pltpu.VMEM((nh * _ROWS, dh), _F32),
            pltpu.VMEM((nb * nh, dh), _F32),
            pltpu.VMEM((nh, _ROWS, dh), _F32),
            pltpu.VMEM((dc // 128, nh * _ROWS, 128), _F32),
            pltpu.VMEM((nb, nh, dc), _F32),
            pltpu.VMEM((sk // _KC, nh, _KC), _F32),
            pltpu.SemaphoreType.DMA((9,)),
        ],
        compiler_params=pltpu.CompilerParams(vmem_limit_bytes=100 * 1024 * 1024, **_PARAMS),
        name="mha_cla_decode",
    )(*operands)
    return out.reshape(nb, sq, 2 * dm)
```

```python
import jax
import jax.numpy as jnp
from jax import lax
import jax.experimental.pallas as pl
import jax.experimental.pallas.tpu as pltpu

_F32 = jnp.float32
_BF16 = jnp.bfloat16
_ROWS = 8
_RING = 4
_KB = 512
_KC = 1024
_SEG = 8192
_WIDE = _SEG // _ROWS
_LAST = 1536
_PRIME = 3
_PARAMS = dict()


def _dot(a, b):
    return lax.dot_general(a, b, (((1,), (0,)), ((), ())), preferred_element_type=_F32)


def _dot_nt(a, b):
    return lax.dot_general(a, b, (((1,), (1,)), ((), ())), preferred_element_type=_F32)


def _divmod(i, n):
    return i >> (n.bit_length() - 1), i & (n - 1)


def _span(start, size):
    return pl.ds(pl.multiple_of(start, size), size)


def _segment(s, cols):
    if cols <= _WIDE:
        return (_span(s * (_SEG // cols), _SEG // cols),)
    r, c = _divmod(s, cols // _WIDE)
    return _span(r * _ROWS, _ROWS), _span(c * _WIDE, _WIDE)


def _eight_heads(w_ref, g, heads):
    stride = heads // 2
    rows = w_ref.shape[1] // heads
    words = w_ref.bitcast(jnp.uint32).at[:, pl.ds(pl.multiple_of(4 * g, 4), (rows - 1) * stride + 4)]
    for j in range(4):
        w = jnp.concatenate([words[i, pl.ds(j, rows, stride=stride), :] for i in range(2)], axis=0)
        yield lax.bitcast_convert_type(w << 16, _F32).astype(_BF16)
        yield lax.bitcast_convert_type((w >> 16) << 16, _F32).astype(_BF16)


def _pad_rows(x):
    x = x.astype(_F32)
    pad = jnp.zeros((_ROWS - x.shape[0], x.shape[1]), _F32)
    return jnp.concatenate([x, pad], axis=0).astype(_BF16)


def _halves(src, dst, sem, parts=4):
    _, rows, cols = src.shape
    stretch = rows * cols // _SEG // parts

    def piece(t, u):
        s = u % parts * stretch + t * (4 // parts) + u // parts
        idx = (slice(None),) + _segment(s, cols)
        return pltpu.make_async_copy(src.at[idx], dst.at[idx], sem)
    return piece


def _request(hi, lo, first, rounds, priority=0):
    def body(t, carry):
        for u in range(4):
            hi(first + t, u).start(priority=priority)
            lo(first + t, u).start(priority=1)
        return carry
    lax.fori_loop(0, rounds, body, 0)


def _arrived(buf, sem):
    pltpu.make_async_copy(buf, buf, sem).wait()


def _kernel(xa_hbm, k_hbm, v_hbm, wqa_hbm, woa_hbm,
            xb_hbm, c_hbm, wqb_hbm, wuk_hbm, wuv_hbm, wob_hbm,
            out_ref,
            xa_v, xb_v, kv_v, wqa_v, woa_v, c_v, wqb_v, wuk_v, wuv_v, wob_v,
            hd_s, qt_s, qb_s, lat_s, bat_s, sc_s,
            sem):
    nb, dm = xa_hbm.shape
    _, sk, dh = k_hbm.shape
    nh = k_hbm.shape[0] // nb
    dc = c_hbm.shape[3]
    ncc = dc // 128
    nkb = sk // _KB
    ngrp = nh // _ROWS
    nsteps = nb * ngrp * nkb
    scale = dh ** -0.5

    wqb_sem, wqa_sem, wuk_sem, wuv_sem, x_sem = (sem.at[n] for n in (0, 1, 2, 3, 7))
    c_sem = lambda b: sem.at[4 + b]
    wob_sem = sem.at[4]

    wqb, wqa = _halves(wqb_hbm, wqb_v, wqb_sem), _halves(wqa_hbm, wqa_v, wqa_sem)
    wuk, wuv = _halves(wuk_hbm, wuk_v, wuk_sem), _halves(wuv_hbm, wuv_v, wuv_sem)
    lat = [_halves(c_hbm.at[b], c_v.at[b], c_sem(b)) for b in range(nb)]
    wob = [_halves(wob_hbm.at[n], wob_v.at[n], wob_sem, 2) for n in range(2)]

    def request_step(i, first=0, rounds=_KB * dh // _SEG):
        grp, kb = _divmod(i, nkb)
        slot = i & (_RING - 1)
        n = _SEG // dh

        def cache(src, which):
            def piece(t, u):
                return pltpu.make_async_copy(
                    src.at[pl.ds(grp * _ROWS + 2 * u, 2), _span(kb * _KB + t * n, n)],
                    kv_v.at[slot, which, pl.ds(2 * u, 2), _span(t * n, n)], sem.at[slot])
            return piece
        _request(cache(k_hbm, 0), cache(v_hbm, 1), first, rounds)

    def woa_hi(t, u):
        idx = (pl.ds(2 * (u % 2), 2),) + _segment(2 * t + u // 2, nh * dh)
        return pltpu.make_async_copy(woa_hbm.at[idx], woa_v.at[idx], sem.at[4])

    def woa_lo(t, u):
        n, t = _divmod(t, 8)
        idx = (pl.ds(4 + 2 * n, 2),) + _segment(4 * t + u, nh * dh)
        return pltpu.make_async_copy(woa_hbm.at[idx], woa_v.at[idx], sem.at[5 + n])

    if _PRIME:
        _request(wqb, wqa, 0, _PRIME, priority=1)
    _request(wqb, wqa, _PRIME, 36 - _PRIME)
    x_copies = [pltpu.make_async_copy(xb_hbm, xb_v, x_sem), pltpu.make_async_copy(xa_hbm, xa_v, x_sem)]
    for copy in x_copies:
        copy.start()
    _request(wuk, wuv, 0, 8)

    for copy in x_copies:
        copy.wait()
    _arrived(wqb_v, wqb_sem)
    xb = _pad_rows(xb_v[...])

    def qb_group(g, carry):
        for e, w in enumerate(_eight_heads(wqb_v, g, nh)):
            qb_s[8 * g + e] = _dot(xb, w)
        _request(wuk, wuv, 8 + 4 * g, 4)
        return carry

    lax.fori_loop(0, ngrp, qb_group, 0)
    _arrived(wqa_v, wqa_sem)
    xa = _pad_rows(xa_v[...])

    def qa_group(g, carry):
        q = _dot(xa, wqa_v[:, :, _span(g * _ROWS * dh, _ROWS * dh)].reshape(dm, _ROWS * dh))
        for e in range(_ROWS):
            hd_s[_span((g * _ROWS + e) * _ROWS, _ROWS), :] = q[:, e * dh:(e + 1) * dh]
        _request(wuk, wuv, 24 + 2 * g, 2)
        return carry

    lax.fori_loop(0, ngrp, qa_group, 0)
    for b in range(nb):
        qt_s[b * nh:(b + 1) * nh, :] = hd_s[pl.ds(b, nh, stride=_ROWS), :]

    _request(lat[0], lat[1], 0, 16)
    _arrived(wuk_v, wuk_sem)
    _arrived(wuv_v, wuv_sem)

    def absorb_group(g, carry):
        for e, w in enumerate(_eight_heads(wuk_v, g, nh)):
            h = 8 * g + e
            r = _dot_nt(qb_s[h].astype(_BF16), w)
            for c in range(ncc):
                lat_s[c, _span(h * _ROWS, _ROWS), :] = r[:, c * 128:(c + 1) * 128]
        _request(lat[0], lat[1], 16 + 4 * g, 4)
        return carry

    lax.fori_loop(0, ngrp, absorb_group, 0)
    for b in range(nb):
        rows = pl.ds(b, nh, stride=_ROWS)
        bat_s[b] = jnp.concatenate([lat_s[c, rows, :] for c in range(ncc)], axis=1)

    nkc = sk // _KC

    def latent_attention(b, carry):
        def request(first, rounds):
            @pl.when(b < 2)
            def _():
                _request(lat[2], lat[3], 8 + 12 * b + first, rounds)

            @pl.when(b == 2)
            def _():
                _request(wob[0], wob[1], 6 + first, rounds)

            @pl.when(b == 3)
            def _():
                request_step(*_divmod(first, 8), rounds)

        @pl.when(b == 0)
        def _():
            _request(lat[2], lat[3], 0, 8)

        @pl.when(b == 2)
        def _():
            _request(wob[0], wob[1], 0, 6)

        _arrived(c_v.at[b], c_sem(b))
        q = bat_s[b].astype(_BF16)

        def latents(t):
            half, chunk = _divmod(t, nkc // 2)
            return c_v[b, half, _span(chunk * _KC, _KC), :]

        def scores(t, m):
            s = _dot_nt(q, latents(t)) * scale
            sc_s[t] = s
            for c in range(_KC // 128):
                m = jnp.maximum(m, s[:, c * 128:(c + 1) * 128])
            request(2 * t, 2)
            return m

        m = lax.fori_loop(0, nkc, scores, jnp.full((nh, 128), -jnp.inf, _F32))
        m = jnp.max(m, axis=1, keepdims=True)

        def context(t, lo):
            l, o = lo
            p = jnp.exp(sc_s[t] - m)
            for c in range(_KC // 128):
                l = l + p[:, c * 128:(c + 1) * 128]
            o = o + _dot(p.astype(_BF16), latents(t))
            request(2 * nkc + t, 1)
            return l, o

        l, o = lax.fori_loop(0, nkc, context,
                             (jnp.zeros((nh, 128), _F32), jnp.zeros((nh, dc), _F32)))
        bat_s[b] = o / jnp.sum(l, axis=1, keepdims=True)
        return carry

    lax.fori_loop(0, nb, latent_attention, 0)
    for b in range(nb):
        rows = pl.ds(b, nh, stride=_ROWS)
        for c in range(ncc):
            lat_s[c, rows, :] = bat_s[b, :, c * 128:(c + 1) * 128]

    request_step(1, 4, 4)

    def value_group(g, carry):
        for e, w in enumerate(_eight_heads(wuv_v, g, nh)):
            h = 8 * g + e
            x = jnp.concatenate([lat_s[c, _span(h * _ROWS, _ROWS), :] for c in range(ncc)], axis=1)
            qb_s[h] = _dot(x.astype(_BF16), w)
        request_step(2, 2 * g, 2)
        return carry

    lax.fori_loop(0, ngrp, value_group, 0)
    _arrived(wob_v, wob_sem)

    def out_group(g, acc):
        n, half = _divmod(g, 2)
        for e in range(_ROWS):
            w = wob_v[n, half, e * dm:(e + 1) * dm, :]
            acc = acc + _dot_nt(qb_s[_ROWS * g + e].astype(_BF16), w)
        request_step(3, 2 * g, 2)
        return acc

    out_b = lax.fori_loop(0, ngrp, out_group, jnp.zeros((_ROWS, dm), _F32))
    out_ref[:, dm:] = out_b[:nb].astype(out_ref.dtype)

    row = lax.broadcasted_iota(jnp.int32, (_ROWS, _KB), 0)

    def group(grp, carry):
        q = qt_s[_span(grp * _ROWS, _ROWS), :].astype(_BF16)

        def step(kb, state):
            m, l, acc = state
            i = grp * nkb + kb
            slot = i & (_RING - 1)
            _arrived(kv_v.at[slot], sem.at[slot])
            full = _dot_nt(q, kv_v[slot, 0].reshape(_ROWS * _KB, dh))
            s = full[:, :_KB]
            for e in range(1, _ROWS):
                s = jnp.where(row == e, full[:, e * _KB:(e + 1) * _KB], s)
            s = s * scale
            m_new = jnp.maximum(m, jnp.max(s, axis=1, keepdims=True))
            alpha = jnp.exp(m - m_new)
            p = jnp.exp(s - m_new)
            l = alpha * l + jnp.sum(p, axis=1, keepdims=True)
            spread = jnp.concatenate([jnp.where(row == e, p, 0.0) for e in range(_ROWS)], axis=1)
            acc = alpha * acc + _dot(spread.astype(_BF16), kv_v[slot, 1].reshape(_ROWS * _KB, dh))

            @pl.when(i + _RING < nsteps)
            def _():
                request_step((i + _RING) & (nsteps - 1))

            @pl.when(i + _RING >= nsteps)
            def _():
                _request(woa_hi, woa_lo, slot * 4, 4)

            return m_new, l, acc

        _, l, acc = lax.fori_loop(
            0, nkb, step,
            (jnp.full((_ROWS, 1), -jnp.inf, _F32), jnp.zeros((_ROWS, 1), _F32),
             jnp.zeros((_ROWS, dh), _F32)))
        qt_s[_span(grp * _ROWS, _ROWS), :] = acc / l
        return carry

    lax.fori_loop(0, nb * ngrp, group, 0)
    tails = [slice(0, nh * dh - _LAST), slice(nh * dh - _LAST, nh * dh)]
    tail_copies = [pltpu.make_async_copy(woa_hbm.at[8, :, cols], woa_v.at[8, :, cols], sem.at[n])
                   for n, cols in enumerate(tails)]
    for copy in tail_copies:
        copy.start(priority=1)

    for b in range(nb):
        hd_s[pl.ds(b, nh, stride=_ROWS), :] = qt_s[b * nh:(b + 1) * nh, :]
    o = jnp.concatenate([hd_s[h * _ROWS:(h + 1) * _ROWS, :] for h in range(nh)], axis=1)
    o = o.astype(_BF16)
    for n, lo, hi in ((5, 4, 6), (4, 0, 4), (6, 6, 8)):
        _arrived(woa_v.at[lo:hi], sem.at[n])
        w = woa_v[lo:hi].reshape((hi - lo) * 64, nh * dh)
        out_ref[:, lo * 64:hi * 64] = _dot_nt(o, w)[:nb].astype(out_ref.dtype)
    tail_copies[0].wait()
    qb_s[0, :, :64] = _dot_nt(o[:, tails[0]], woa_v[8, :, tails[0]])
    tail_copies[1].wait()
    rest = qb_s[0, :, :64] + _dot_nt(o[:, tails[1]], woa_v[8, :, tails[1]])
    out_ref[:, dm - 64:dm] = rest[:nb].astype(out_ref.dtype)


@jax.jit
def pallas_concat_heads__mha_block_cached__compressed_kv_cla__decode_kernel(
    A_x: jax.Array,
    A_k_cache: jax.Array,
    A_v_cache: jax.Array,
    A_wq: jax.Array,
    A_wo: jax.Array,
    B_x: jax.Array,
    B_c_kv: jax.Array,
    B_w_q: jax.Array,
    B_w_uk: jax.Array,
    B_w_uv: jax.Array,
    B_w_o: jax.Array,
):
    nb, sq, dm = A_x.shape
    _, nh, sk, dh = A_k_cache.shape
    dc = B_c_kv.shape[2]
    assert (nb, sq, dm, nh, sk, dh, dc) == (4, 1, 576, 32, 4096, 128, 512)

    xa, xb = A_x.reshape(nb, dm), B_x.reshape(nb, dm)
    k, v = A_k_cache.reshape(nb * nh, sk, dh), A_v_cache.reshape(nb * nh, sk, dh)
    wqa = A_wq.reshape(2, dm // 2, nh * dh)
    woa = A_wo.T.reshape(dm // 64, 64, nh * dh)
    c = B_c_kv.reshape(nb, 2, sk // 2, dc)
    wqb = B_w_q.reshape(2, dm // 2 * nh, dh)
    wuk = B_w_uk.reshape(2, dc // 2 * nh, dh)
    wuv = B_w_uv.reshape(2, dc // 2 * nh, dh)
    wob = B_w_o.transpose(0, 2, 1).reshape(2, 2, nh // 4 * dm, dh)
    operands = (xa, k, v, wqa, woa, xb, c, wqb, wuk, wuv, wob)

    like = lambda a: pltpu.VMEM(a.shape, a.dtype)
    out = pl.pallas_call(
        _kernel,
        in_specs=[pl.BlockSpec(memory_space=pl.ANY)] * len(operands),
        out_specs=pl.BlockSpec(memory_space=pltpu.VMEM),
        out_shape=jax.ShapeDtypeStruct((nb, 2 * dm), A_x.dtype),
        scratch_shapes=[
            like(xa), like(xb), pltpu.VMEM((_RING, 2, _ROWS, _KB, dh), k.dtype),
            like(wqa), like(woa), like(c), like(wqb), like(wuk), like(wuv), like(wob),
            pltpu.VMEM((nh * _ROWS, dh), _F32),
            pltpu.VMEM((nb * nh, dh), _F32),
            pltpu.VMEM((nh, _ROWS, dh), _F32),
            pltpu.VMEM((dc // 128, nh * _ROWS, 128), _F32),
            pltpu.VMEM((nb, nh, dc), _F32),
            pltpu.VMEM((sk // _KC, nh, _KC), _F32),
            pltpu.SemaphoreType.DMA((8,)),
        ],
        compiler_params=pltpu.CompilerParams(vmem_limit_bytes=100 * 1024 * 1024, **_PARAMS),
        name="mha_cla_decode",
    )(*operands)
    return out.reshape(nb, sq, 2 * dm)
```

```python
import jax
import jax.numpy as jnp
import numpy as np
from jax import lax
import jax.experimental.pallas as pl
import jax.experimental.pallas.tpu as pltpu

_F32 = jnp.float32
_BF16 = jnp.bfloat16
_LOWEST = float(np.finfo(np.float32).min)
_ROWS = 8
_RING = 4
_KB = 512
_KC = 1024
_SEG = 8192
_WIDE = _SEG // _ROWS
_BLOCK = 64
_LAST = 1536


def _dot(a, b):
    return lax.dot_general(a, b, (((1,), (0,)), ((), ())), preferred_element_type=_F32)


def _dot_nt(a, b):
    return lax.dot_general(a, b, (((1,), (1,)), ((), ())), preferred_element_type=_F32)


def _divmod(i, n):
    return i >> (n.bit_length() - 1), i & (n - 1)


def _span(start, size):
    return pl.ds(pl.multiple_of(start, size), size)


def _segment(s, cols):
    if cols <= _WIDE:
        return (_span(s * (_SEG // cols), _SEG // cols),)
    r, c = _divmod(s, cols // _WIDE)
    return _span(r * _ROWS, _ROWS), _span(c * _WIDE, _WIDE)


def _halves(src, dst, sem, parts=4):
    _, rows, cols = src.shape
    stretch = rows * cols // _SEG // parts

    def piece(t, u):
        s = u % parts * stretch + t * (4 // parts) + u // parts
        idx = (slice(None),) + _segment(s, cols)
        return pltpu.make_async_copy(src.at[idx], dst.at[idx], sem)
    return piece


def _request(hi, lo, first, rounds, priority=0):
    def body(t, carry):
        for u in range(4):
            hi(first + t, u).start(priority=priority)
            lo(first + t, u).start(priority=1)
        return carry
    lax.fori_loop(0, rounds, body, 0)


def _arrived(buf, sem):
    pltpu.make_async_copy(buf, buf, sem).wait()


def _eight_heads(w_ref, g, heads):
    stride = heads // 2
    rows = w_ref.shape[1] // heads
    window = pl.ds(pl.multiple_of(4 * g, 4), (rows - 1) * stride + 4)
    words = w_ref.bitcast(jnp.uint32).at[:, window]
    for j in range(4):
        w = jnp.concatenate([words[i, pl.ds(j, rows, stride=stride), :] for i in range(2)], axis=0)
        yield lax.bitcast_convert_type(w << 16, _F32).astype(_BF16)
        yield lax.bitcast_convert_type((w >> 16) << 16, _F32).astype(_BF16)


def _pad_rows(x):
    x = x.astype(_F32)
    pad = jnp.zeros((_ROWS - x.shape[0], x.shape[1]), _F32)
    return jnp.concatenate([x, pad], axis=0).astype(_BF16)


def _body(xa_hbm, k_hbm, v_hbm, wqa_hbm, woa_hbm,
          xb_hbm, c_hbm, wqb_hbm, wuk_hbm, wuv_hbm, wob_hbm,
          out_ref,
          xa_v, xb_v, kv_v, wqa_v, woa_v, c_v, wqb_v, wuk_v, wuv_v, wob_v,
          head_s,
          batch_s,
          qb_s,
          lat_s,
          bat_s,
          sc_s,
          rest_s,
          sem):
    nb, dm = xa_hbm.shape
    _, sk, dh = k_hbm.shape
    nh = k_hbm.shape[0] // nb
    dc = c_hbm.shape[3]
    ncc = dc // 128
    nkb = sk // _KB
    nkc = sk // _KC
    ngrp = nh // _ROWS
    nsteps = nb * ngrp * nkb
    scale = dh ** -0.5

    c_sem = lambda b: sem.at[_RING + b]
    woa_sem = lambda n: sem.at[_RING + nb + n]
    xa_sem, xb_sem, wqa_sem, wqb_sem, wuk_sem, wuv_sem, wob_sem = (
        sem.at[_RING + nb + 5 + n] for n in range(7))

    wqb, wqa = _halves(wqb_hbm, wqb_v, wqb_sem), _halves(wqa_hbm, wqa_v, wqa_sem)
    wuk, wuv = _halves(wuk_hbm, wuk_v, wuk_sem), _halves(wuv_hbm, wuv_v, wuv_sem)
    lat = [_halves(c_hbm.at[b], c_v.at[b], c_sem(b)) for b in range(nb)]
    wob = [_halves(wob_hbm.at[n], wob_v.at[n], wob_sem, 2) for n in range(2)]

    def request_step(i, first=0, rounds=_KB * dh // _SEG):
        grp, kb = _divmod(i, nkb)
        slot = i & (_RING - 1)
        n = _SEG // dh

        def cache(src, which):
            def piece(t, u):
                return pltpu.make_async_copy(
                    src.at[pl.ds(grp * _ROWS + 2 * u, 2), _span(kb * _KB + t * n, n)],
                    kv_v.at[slot, which, pl.ds(2 * u, 2), _span(t * n, n)], sem.at[slot])
            return piece
        _request(cache(k_hbm, 0), cache(v_hbm, 1), first, rounds)

    def woa_hi(t, u):
        idx = (pl.ds(2 * (u % 2), 2),) + _segment(2 * t + u // 2, nh * dh)
        return pltpu.make_async_copy(woa_hbm.at[idx], woa_v.at[idx], woa_sem(0))

    def woa_lo(t, u):
        n, t = _divmod(t, 8)
        idx = (pl.ds(4 + 2 * n, 2),) + _segment(4 * t + u, nh * dh)
        return pltpu.make_async_copy(woa_hbm.at[idx], woa_v.at[idx], woa_sem(1 + n))

    _request(wqb, wqa, 0, 3, priority=1)
    _request(wqb, wqa, 3, 33)
    xb_copy = pltpu.make_async_copy(xb_hbm, xb_v, xb_sem)
    xa_copy = pltpu.make_async_copy(xa_hbm, xa_v, xa_sem)
    xb_copy.start()
    xa_copy.start()
    _request(wuk, wuv, 0, 8)

    xb_copy.wait()
    _arrived(wqb_v, wqb_sem)
    xb = _pad_rows(xb_v[...])

    def qb_group(g, carry):
        for e, w in enumerate(_eight_heads(wqb_v, g, nh)):
            qb_s[_ROWS * g + e] = _dot(xb, w)
        _request(wuk, wuv, 8 + 4 * g, 4)
        return carry

    lax.fori_loop(0, ngrp, qb_group, 0)
    xa_copy.wait()
    _arrived(wqa_v, wqa_sem)
    xa = _pad_rows(xa_v[...])

    def qa_group(g, carry):
        q = _dot(xa, wqa_v[:, :, _span(g * _ROWS * dh, _ROWS * dh)].reshape(dm, _ROWS * dh))
        for e in range(_ROWS):
            head_s[_span((_ROWS * g + e) * _ROWS, _ROWS), :] = q[:, e * dh:(e + 1) * dh]
        _request(wuk, wuv, 24 + 2 * g, 2)
        return carry

    lax.fori_loop(0, ngrp, qa_group, 0)
    for b in range(nb):
        batch_s[b * nh:(b + 1) * nh, :] = head_s[pl.ds(b, nh, stride=_ROWS), :]

    _request(lat[0], lat[1], 0, 16)
    _arrived(wuk_v, wuk_sem)

    def absorb_group(g, carry):
        for e, w in enumerate(_eight_heads(wuk_v, g, nh)):
            h = _ROWS * g + e
            r = _dot_nt(qb_s[h].astype(_BF16), w)
            for c in range(ncc):
                lat_s[c, _span(h * _ROWS, _ROWS), :] = r[:, c * 128:(c + 1) * 128]
        _request(lat[0], lat[1], 16 + 4 * g, 4)
        return carry

    lax.fori_loop(0, ngrp, absorb_group, 0)
    for b in range(nb):
        rows = pl.ds(b, nh, stride=_ROWS)
        bat_s[b] = jnp.concatenate([lat_s[c, rows, :] for c in range(ncc)], axis=1)

    def latent_attention(b, carry):
        def request(first, rounds):
            @pl.when(b < 2)
            def _():
                _request(lat[2], lat[3], 8 + 12 * b + first, rounds)

            @pl.when(b == 2)
            def _():
                _request(wob[0], wob[1], 6 + first, rounds)

            @pl.when(b == 3)
            def _():
                request_step(*_divmod(first, 8), rounds)

        @pl.when(b == 0)
        def _():
            _request(lat[2], lat[3], 0, 8)

        @pl.when(b == 2)
        def _():
            _request(wob[0], wob[1], 0, 6)

        _arrived(c_v.at[b], c_sem(b))
        q = bat_s[b].astype(_BF16)

        def latents(t):
            half, chunk = _divmod(t, nkc // 2)
            return c_v[b, half, _span(chunk * _KC, _KC), :]

        def scores(t, m):
            s = _dot_nt(q, latents(t)) * scale
            sc_s[t] = s
            for c in range(_KC // 128):
                m = jnp.maximum(m, s[:, c * 128:(c + 1) * 128])
            request(2 * t, 2)
            return m

        m = lax.fori_loop(0, nkc, scores, jnp.full((nh, 128), _LOWEST, _F32))
        m = jnp.max(m, axis=1, keepdims=True)

        def context(t, state):
            l, o = state
            p = jnp.exp(sc_s[t] - m)
            for c in range(_KC // 128):
                l = l + p[:, c * 128:(c + 1) * 128]
            o = o + _dot(p.astype(_BF16), latents(t))
            request(2 * nkc + t, 1)
            return l, o

        l, o = lax.fori_loop(0, nkc, context,
                             (jnp.zeros((nh, 128), _F32), jnp.zeros((nh, dc), _F32)))
        bat_s[b] = o / jnp.sum(l, axis=1, keepdims=True)
        return carry

    lax.fori_loop(0, nb, latent_attention, 0)
    for b in range(nb):
        rows = pl.ds(b, nh, stride=_ROWS)
        for c in range(ncc):
            lat_s[c, rows, :] = bat_s[b, :, c * 128:(c + 1) * 128]

    request_step(1, 4, 4)
    _arrived(wuv_v, wuv_sem)

    def value_group(g, carry):
        for e, w in enumerate(_eight_heads(wuv_v, g, nh)):
            h = _ROWS * g + e
            x = jnp.concatenate([lat_s[c, _span(h * _ROWS, _ROWS), :] for c in range(ncc)], axis=1)
            qb_s[h] = _dot(x.astype(_BF16), w)
        request_step(2, 2 * g, 2)
        return carry

    lax.fori_loop(0, ngrp, value_group, 0)
    _arrived(wob_v, wob_sem)

    def out_group(g, acc):
        n, half = _divmod(g, 2)
        for e in range(_ROWS):
            w = wob_v[n, half, e * dm:(e + 1) * dm, :]
            acc = acc + _dot_nt(qb_s[_ROWS * g + e].astype(_BF16), w)
        request_step(3, 2 * g, 2)
        return acc

    out_b = lax.fori_loop(0, ngrp, out_group, jnp.zeros((_ROWS, dm), _F32))
    out_ref[:, dm:] = out_b[:nb].astype(out_ref.dtype)

    row = lax.broadcasted_iota(jnp.int32, (_ROWS, _KB), 0)

    def group(grp, carry):
        q = batch_s[_span(grp * _ROWS, _ROWS), :].astype(_BF16)

        def step(kb, state):
            m, l, acc = state
            i = grp * nkb + kb
            slot = i & (_RING - 1)
            _arrived(kv_v.at[slot], sem.at[slot])
            full = _dot_nt(q, kv_v[slot, 0].reshape(_ROWS * _KB, dh))
            s = full[:, :_KB]
            for e in range(1, _ROWS):
                s = jnp.where(row == e, full[:, e * _KB:(e + 1) * _KB], s)
            s = s * scale
            m_new = jnp.maximum(m, jnp.max(s, axis=1, keepdims=True))
            alpha = jnp.exp(m - m_new)
            p = jnp.exp(s - m_new)
            l = alpha * l + jnp.sum(p, axis=1, keepdims=True)
            spread = jnp.concatenate([jnp.where(row == e, p, 0.0) for e in range(_ROWS)], axis=1)
            acc = alpha * acc + _dot(spread.astype(_BF16), kv_v[slot, 1].reshape(_ROWS * _KB, dh))

            @pl.when(i + _RING < nsteps)
            def _():
                request_step((i + _RING) & (nsteps - 1))

            @pl.when(i + _RING >= nsteps)
            def _():
                _request(woa_hi, woa_lo, slot * 4, 4)

            return m_new, l, acc

        _, l, acc = lax.fori_loop(
            0, nkb, step,
            (jnp.full((_ROWS, 1), _LOWEST, _F32), jnp.zeros((_ROWS, 1), _F32),
             jnp.zeros((_ROWS, dh), _F32)))
        batch_s[_span(grp * _ROWS, _ROWS), :] = acc / l
        return carry

    lax.fori_loop(0, nb * ngrp, group, 0)

    last = woa_v.shape[0] - 1
    left, right = slice(0, nh * dh - _LAST), slice(nh * dh - _LAST, nh * dh)
    left_copy, right_copy = (
        pltpu.make_async_copy(woa_hbm.at[last, :, cols], woa_v.at[last, :, cols], woa_sem(n))
        for n, cols in ((3, left), (4, right)))
    left_copy.start(priority=1)
    right_copy.start(priority=1)

    for b in range(nb):
        head_s[pl.ds(b, nh, stride=_ROWS), :] = batch_s[b * nh:(b + 1) * nh, :]
    o = jnp.concatenate([head_s[h * _ROWS:(h + 1) * _ROWS, :] for h in range(nh)], axis=1)
    o = o.astype(_BF16)
    for n, lo, hi in ((1, 4, 6), (0, 0, 4), (2, 6, 8)):
        _arrived(woa_v.at[lo:hi], woa_sem(n))
        w = woa_v[lo:hi].reshape((hi - lo) * _BLOCK, nh * dh)
        out_ref[:, lo * _BLOCK:hi * _BLOCK] = _dot_nt(o, w)[:nb].astype(out_ref.dtype)
    left_copy.wait()
    rest_s[...] = _dot_nt(o[:, left], woa_v[last, :, left])
    right_copy.wait()
    rest = rest_s[...] + _dot_nt(o[:, right], woa_v[last, :, right])
    out_ref[:, last * _BLOCK:dm] = rest[:nb].astype(out_ref.dtype)


def _kernel(*refs):
    pl.run_scoped(lambda sem: _body(*refs, sem), pltpu.SemaphoreType.DMA((20,)))


@jax.jit
def pallas_concat_heads__mha_block_cached__compressed_kv_cla__decode_kernel(
    A_x: jax.Array,
    A_k_cache: jax.Array,
    A_v_cache: jax.Array,
    A_wq: jax.Array,
    A_wo: jax.Array,
    B_x: jax.Array,
    B_c_kv: jax.Array,
    B_w_q: jax.Array,
    B_w_uk: jax.Array,
    B_w_uv: jax.Array,
    B_w_o: jax.Array,
):
    nb, sq, dm = A_x.shape
    _, nh, sk, dh = A_k_cache.shape
    dc = B_c_kv.shape[2]
    assert (nb, sq, dm, nh, sk, dh, dc) == (4, 1, 576, 32, 4096, 128, 512)

    xa, xb = A_x.reshape(nb, dm), B_x.reshape(nb, dm)
    k, v = A_k_cache.reshape(nb * nh, sk, dh), A_v_cache.reshape(nb * nh, sk, dh)
    wqa = A_wq.reshape(2, dm // 2, nh * dh)
    woa = A_wo.T.reshape(dm // _BLOCK, _BLOCK, nh * dh)
    c = B_c_kv.reshape(nb, 2, sk // 2, dc)
    wqb = B_w_q.reshape(2, dm // 2 * nh, dh)
    wuk = B_w_uk.reshape(2, dc // 2 * nh, dh)
    wuv = B_w_uv.reshape(2, dc // 2 * nh, dh)
    wob = B_w_o.transpose(0, 2, 1).reshape(2, 2, nh // 4 * dm, dh)
    operands = (xa, k, v, wqa, woa, xb, c, wqb, wuk, wuv, wob)
    assert all(a.dtype == _BF16 for a in operands)

    like = lambda a: pltpu.VMEM(a.shape, a.dtype)
    out = pl.pallas_call(
        _kernel,
        in_specs=[pl.BlockSpec(memory_space=pl.ANY)] * len(operands),
        out_specs=pl.BlockSpec(memory_space=pltpu.VMEM),
        out_shape=jax.ShapeDtypeStruct((nb, 2 * dm), A_x.dtype),
        scratch_shapes=[
            like(xa), like(xb), pltpu.VMEM((_RING, 2, _ROWS, _KB, dh), k.dtype),
            like(wqa), like(woa), like(c), like(wqb), like(wuk), like(wuv), like(wob),
            pltpu.VMEM((nh * _ROWS, dh), _F32),
            pltpu.VMEM((nb * nh, dh), _F32),
            pltpu.VMEM((nh, _ROWS, dh), _F32),
            pltpu.VMEM((dc // 128, nh * _ROWS, 128), _F32),
            pltpu.VMEM((nb, nh, dc), _F32),
            pltpu.VMEM((sk // _KC, nh, _KC), _F32),
            pltpu.VMEM((_ROWS, _BLOCK), _F32),
        ],
        compiler_params=pltpu.CompilerParams(vmem_limit_bytes=100 * 1024 * 1024),
        name="mha_cla_decode",
    )(*operands)
    return out.reshape(nb, sq, 2 * dm)
```

```python
import math

import jax
import jax.numpy as jnp
import numpy as np
from jax import lax
import jax.experimental.pallas as pl
import jax.experimental.pallas.tpu as pltpu

_F32 = jnp.float32
_BF16 = jnp.bfloat16
_LOWEST = float(np.finfo(np.float32).min)
_ROWS = 8
_RING = 4
_KB = 512
_KC = 1024
_SEG = 8192
_WIDE = _SEG // _ROWS
_BLOCK = 64
_LAST = 1536


def _dot(a, b):
    return lax.dot_general(a, b, (((1,), (0,)), ((), ())), preferred_element_type=_F32)


def _dot_nt(a, b):
    return lax.dot_general(a, b, (((1,), (1,)), ((), ())), preferred_element_type=_F32)


def _divmod(i, n):
    return i >> (n.bit_length() - 1), i & (n - 1)


def _span(start, size):
    return pl.ds(pl.multiple_of(start, size), size)


def _segment(s, row_shape):
    if row_shape[-1] <= _WIDE:
        n = _SEG // math.prod(row_shape)
        return (_span(s * n, n),)
    r, c = _divmod(s, row_shape[-1] // _WIDE)
    return _span(r * _ROWS, _ROWS), _span(c * _WIDE, _WIDE)


def _halves(src, dst, sem, parts=4):
    stretch = math.prod(src.shape[1:]) // _SEG // parts

    def piece(t, u):
        s = u % parts * stretch + t * (4 // parts) + u // parts
        idx = (slice(None),) + _segment(s, src.shape[2:])
        return pltpu.make_async_copy(src.at[idx], dst.at[idx], sem)
    return piece


def _request(hi, lo, first, rounds, priority=0):
    def body(t, carry):
        for u in range(4):
            hi(first + t, u).start(priority=priority)
            lo(first + t, u).start(priority=1)
        return carry
    lax.fori_loop(0, rounds, body, 0)


def _arrived(buf, sem):
    pltpu.make_async_copy(buf, buf, sem).wait()


def _eight_heads(w_ref, g, tmp_s):
    w = w_ref[:, :, _span(g * _ROWS, _ROWS), :].astype(_F32)
    rows = w.shape[0] * w.shape[1]
    tmp_s[:rows * _ROWS, :] = w.reshape(rows * _ROWS, w.shape[3])
    for e in range(_ROWS):
        yield tmp_s[pl.ds(e, rows, stride=_ROWS), :].astype(_BF16)


def _pad_rows(x):
    x = x.astype(_F32)
    pad = jnp.zeros((_ROWS - x.shape[0], x.shape[1]), _F32)
    return jnp.concatenate([x, pad], axis=0).astype(_BF16)


def _body(xa_hbm, k_hbm, v_hbm, wqa_hbm, woa_hbm,
          xb_hbm, c_hbm, wqb_hbm, wuk_hbm, wuv_hbm, wob_hbm,
          out_ref,
          xa_v, xb_v, kv_v, wqa_v, woa_v, c_v, wqb_v, wuk_v, wuv_v, wob_v,
          head_s,
          batch_s,
          qb_s,
          lat_s,
          bat_s,
          sc_s,
          rest_s,
          tmp_s,
          sem):
    nb, dm = xa_hbm.shape
    _, sk, dh = k_hbm.shape
    nh = k_hbm.shape[0] // nb
    dc = c_hbm.shape[3]
    ncc = dc // 128
    nkb = sk // _KB
    nkc = sk // _KC
    ngrp = nh // _ROWS
    nsteps = nb * ngrp * nkb
    scale = dh ** -0.5

    c_sem = lambda b: sem.at[_RING + b]
    woa_sem = lambda n: sem.at[_RING + nb + n]
    xa_sem, xb_sem, wqa_sem, wqb_sem, wuk_sem, wuv_sem, wob_sem = (
        sem.at[_RING + nb + 5 + n] for n in range(7))

    wqb, wqa = _halves(wqb_hbm, wqb_v, wqb_sem), _halves(wqa_hbm, wqa_v, wqa_sem)
    wuk, wuv = _halves(wuk_hbm, wuk_v, wuk_sem), _halves(wuv_hbm, wuv_v, wuv_sem)
    lat = [_halves(c_hbm.at[b], c_v.at[b], c_sem(b)) for b in range(nb)]
    wob = [_halves(wob_hbm.at[n], wob_v.at[n], wob_sem, 2) for n in range(2)]

    def request_step(i, first=0, rounds=_KB * dh // _SEG):
        grp, kb = _divmod(i, nkb)
        slot = i & (_RING - 1)
        n = _SEG // dh

        def cache(src, which):
            def piece(t, u):
                return pltpu.make_async_copy(
                    src.at[pl.ds(grp * _ROWS + 2 * u, 2), _span(kb * _KB + t * n, n)],
                    kv_v.at[slot, which, pl.ds(2 * u, 2), _span(t * n, n)], sem.at[slot])
            return piece
        _request(cache(k_hbm, 0), cache(v_hbm, 1), first, rounds)

    def woa_hi(t, u):
        idx = (pl.ds(2 * (u % 2), 2),) + _segment(2 * t + u // 2, woa_v.shape[2:])
        return pltpu.make_async_copy(woa_hbm.at[idx], woa_v.at[idx], woa_sem(0))

    def woa_lo(t, u):
        n, t = _divmod(t, 8)
        idx = (pl.ds(4 + 2 * n, 2),) + _segment(4 * t + u, woa_v.shape[2:])
        return pltpu.make_async_copy(woa_hbm.at[idx], woa_v.at[idx], woa_sem(1 + n))

    _request(wqb, wqa, 0, 3, priority=1)
    _request(wqb, wqa, 3, 33)
    xb_copy = pltpu.make_async_copy(xb_hbm, xb_v, xb_sem)
    xa_copy = pltpu.make_async_copy(xa_hbm, xa_v, xa_sem)
    xb_copy.start()
    xa_copy.start()
    _request(wuk, wuv, 0, 8)

    xb_copy.wait()
    _arrived(wqb_v, wqb_sem)
    xb = _pad_rows(xb_v[...])

    def qb_group(g, carry):
        for e, w in enumerate(_eight_heads(wqb_v, g, tmp_s)):
            qb_s[_ROWS * g + e] = _dot(xb, w)
        _request(wuk, wuv, 8 + 4 * g, 4)
        return carry

    lax.fori_loop(0, ngrp, qb_group, 0)
    xa_copy.wait()
    _arrived(wqa_v, wqa_sem)
    xa = _pad_rows(xa_v[...])

    def qa_group(g, carry):
        q = _dot(xa, wqa_v[:, :, _span(g * _ROWS * dh, _ROWS * dh)].reshape(dm, _ROWS * dh))
        for e in range(_ROWS):
            head_s[_span((_ROWS * g + e) * _ROWS, _ROWS), :] = q[:, e * dh:(e + 1) * dh]
        _request(wuk, wuv, 24 + 2 * g, 2)
        return carry

    lax.fori_loop(0, ngrp, qa_group, 0)
    for b in range(nb):
        batch_s[b * nh:(b + 1) * nh, :] = head_s[pl.ds(b, nh, stride=_ROWS), :]

    _request(lat[0], lat[1], 0, 16)
    _arrived(wuk_v, wuk_sem)

    def absorb_group(g, carry):
        for e, w in enumerate(_eight_heads(wuk_v, g, tmp_s)):
            h = _ROWS * g + e
            r = _dot_nt(qb_s[h].astype(_BF16), w)
            for c in range(ncc):
                lat_s[c, _span(h * _ROWS, _ROWS), :] = r[:, c * 128:(c + 1) * 128]
        _request(lat[0], lat[1], 16 + 4 * g, 4)
        return carry

    lax.fori_loop(0, ngrp, absorb_group, 0)
    for b in range(nb):
        rows = pl.ds(b, nh, stride=_ROWS)
        bat_s[b] = jnp.concatenate([lat_s[c, rows, :] for c in range(ncc)], axis=1)

    def latent_attention(b, carry):
        def request(first, rounds):
            @pl.when(b < 2)
            def _():
                _request(lat[2], lat[3], 8 + 12 * b + first, rounds)

            @pl.when(b == 2)
            def _():
                _request(wob[0], wob[1], 6 + first, rounds)

            @pl.when(b == 3)
            def _():
                request_step(*_divmod(first, 8), rounds)

        @pl.when(b == 0)
        def _():
            _request(lat[2], lat[3], 0, 8)

        @pl.when(b == 2)
        def _():
            _request(wob[0], wob[1], 0, 6)

        _arrived(c_v.at[b], c_sem(b))
        q = bat_s[b].astype(_BF16)

        def latents(t):
            half, chunk = _divmod(t, nkc // 2)
            return c_v[b, half, _span(chunk * _KC, _KC), :]

        def scores(t, m):
            s = _dot_nt(q, latents(t)) * scale
            sc_s[t] = s
            for c in range(_KC // 128):
                m = jnp.maximum(m, s[:, c * 128:(c + 1) * 128])
            request(2 * t, 2)
            return m

        m = lax.fori_loop(0, nkc, scores, jnp.full((nh, 128), _LOWEST, _F32))
        m = jnp.max(m, axis=1, keepdims=True)

        def context(t, state):
            l, o = state
            p = jnp.exp(sc_s[t] - m)
            for c in range(_KC // 128):
                l = l + p[:, c * 128:(c + 1) * 128]
            o = o + _dot(p.astype(_BF16), latents(t))
            request(2 * nkc + t, 1)
            return l, o

        l, o = lax.fori_loop(0, nkc, context,
                             (jnp.zeros((nh, 128), _F32), jnp.zeros((nh, dc), _F32)))
        bat_s[b] = o / jnp.sum(l, axis=1, keepdims=True)
        return carry

    lax.fori_loop(0, nb, latent_attention, 0)
    for b in range(nb):
        rows = pl.ds(b, nh, stride=_ROWS)
        for c in range(ncc):
            lat_s[c, rows, :] = bat_s[b, :, c * 128:(c + 1) * 128]

    request_step(1, 4, 4)
    _arrived(wuv_v, wuv_sem)

    def value_group(g, carry):
        for e, w in enumerate(_eight_heads(wuv_v, g, tmp_s)):
            h = _ROWS * g + e
            x = jnp.concatenate([lat_s[c, _span(h * _ROWS, _ROWS), :] for c in range(ncc)], axis=1)
            qb_s[h] = _dot(x.astype(_BF16), w)
        request_step(2, 2 * g, 2)
        return carry

    lax.fori_loop(0, ngrp, value_group, 0)
    _arrived(wob_v, wob_sem)

    def out_group(g, acc):
        n, half = _divmod(g, 2)
        for e in range(_ROWS):
            w = wob_v[n, half, e * dm:(e + 1) * dm, :]
            acc = acc + _dot_nt(qb_s[_ROWS * g + e].astype(_BF16), w)
        request_step(3, 2 * g, 2)
        return acc

    out_b = lax.fori_loop(0, ngrp, out_group, jnp.zeros((_ROWS, dm), _F32))
    out_ref[:, dm:] = out_b[:nb].astype(out_ref.dtype)

    row = lax.broadcasted_iota(jnp.int32, (_ROWS, _KB), 0)

    def group(grp, carry):
        q = batch_s[_span(grp * _ROWS, _ROWS), :].astype(_BF16)

        def step(kb, state):
            m, l, acc = state
            i = grp * nkb + kb
            slot = i & (_RING - 1)
            _arrived(kv_v.at[slot], sem.at[slot])
            full = _dot_nt(q, kv_v[slot, 0].reshape(_ROWS * _KB, dh))
            s = full[:, :_KB]
            for e in range(1, _ROWS):
                s = jnp.where(row == e, full[:, e * _KB:(e + 1) * _KB], s)
            s = s * scale
            m_new = jnp.maximum(m, jnp.max(s, axis=1, keepdims=True))
            alpha = jnp.exp(m - m_new)
            p = jnp.exp(s - m_new)
            l = alpha * l + jnp.sum(p, axis=1, keepdims=True)
            spread = jnp.concatenate([jnp.where(row == e, p, 0.0) for e in range(_ROWS)], axis=1)
            acc = alpha * acc + _dot(spread.astype(_BF16), kv_v[slot, 1].reshape(_ROWS * _KB, dh))

            @pl.when(i + _RING < nsteps)
            def _():
                request_step((i + _RING) & (nsteps - 1))

            @pl.when(i + _RING >= nsteps)
            def _():
                _request(woa_hi, woa_lo, slot * 4, 4)

            return m_new, l, acc

        _, l, acc = lax.fori_loop(
            0, nkb, step,
            (jnp.full((_ROWS, 1), _LOWEST, _F32), jnp.zeros((_ROWS, 1), _F32),
             jnp.zeros((_ROWS, dh), _F32)))
        batch_s[_span(grp * _ROWS, _ROWS), :] = acc / l
        return carry

    lax.fori_loop(0, nb * ngrp, group, 0)

    last = woa_v.shape[0] - 1
    left, right = slice(0, nh * dh - _LAST), slice(nh * dh - _LAST, nh * dh)
    left_copy, right_copy = (
        pltpu.make_async_copy(woa_hbm.at[last, :, cols], woa_v.at[last, :, cols], woa_sem(n))
        for n, cols in ((3, left), (4, right)))
    left_copy.start(priority=1)
    right_copy.start(priority=1)

    for b in range(nb):
        head_s[pl.ds(b, nh, stride=_ROWS), :] = batch_s[b * nh:(b + 1) * nh, :]
    o = jnp.concatenate([head_s[h * _ROWS:(h + 1) * _ROWS, :] for h in range(nh)], axis=1)
    o = o.astype(_BF16)
    for n, lo, hi in ((1, 4, 6), (0, 0, 4), (2, 6, 8)):
        _arrived(woa_v.at[lo:hi], woa_sem(n))
        w = woa_v[lo:hi].reshape((hi - lo) * _BLOCK, nh * dh)
        out_ref[:, lo * _BLOCK:hi * _BLOCK] = _dot_nt(o, w)[:nb].astype(out_ref.dtype)
    left_copy.wait()
    rest_s[...] = _dot_nt(o[:, left], woa_v[last, :, left])
    right_copy.wait()
    rest = rest_s[...] + _dot_nt(o[:, right], woa_v[last, :, right])
    out_ref[:, last * _BLOCK:dm] = rest[:nb].astype(out_ref.dtype)


def _kernel(*refs):
    pl.run_scoped(lambda sem: _body(*refs, sem), pltpu.SemaphoreType.DMA((20,)))


@jax.jit
def pallas_concat_heads__mha_block_cached__compressed_kv_cla__decode_kernel(
    A_x: jax.Array,
    A_k_cache: jax.Array,
    A_v_cache: jax.Array,
    A_wq: jax.Array,
    A_wo: jax.Array,
    B_x: jax.Array,
    B_c_kv: jax.Array,
    B_w_q: jax.Array,
    B_w_uk: jax.Array,
    B_w_uv: jax.Array,
    B_w_o: jax.Array,
):
    nb, sq, dm = A_x.shape
    _, nh, sk, dh = A_k_cache.shape
    dc = B_c_kv.shape[2]
    assert (nb, sq, dm, nh, sk, dh, dc) == (4, 1, 576, 32, 4096, 128, 512)

    xa, xb = A_x.reshape(nb, dm), B_x.reshape(nb, dm)
    k, v = A_k_cache.reshape(nb * nh, sk, dh), A_v_cache.reshape(nb * nh, sk, dh)
    wqa = A_wq.reshape(2, dm // 2, nh * dh)
    woa = A_wo.T.reshape(dm // _BLOCK, _BLOCK, nh * dh)
    c = B_c_kv.reshape(nb, 2, sk // 2, dc)
    wqb = B_w_q.reshape(2, dm // 2, nh, dh)
    wuk = B_w_uk.reshape(2, dc // 2, nh, dh)
    wuv = B_w_uv.reshape(2, dc // 2, nh, dh)
    wob = B_w_o.transpose(0, 2, 1).reshape(2, 2, nh // 4 * dm, dh)
    operands = (xa, k, v, wqa, woa, xb, c, wqb, wuk, wuv, wob)
    assert all(a.dtype == _BF16 for a in operands)

    like = lambda a: pltpu.VMEM(a.shape, a.dtype)
    out = pl.pallas_call(
        _kernel,
        in_specs=[pl.BlockSpec(memory_space=pl.ANY)] * len(operands),
        out_specs=pl.BlockSpec(memory_space=pltpu.VMEM),
        out_shape=jax.ShapeDtypeStruct((nb, 2 * dm), A_x.dtype),
        scratch_shapes=[
            like(xa), like(xb), pltpu.VMEM((_RING, 2, _ROWS, _KB, dh), k.dtype),
            like(wqa), like(woa), like(c), like(wqb), like(wuk), like(wuv), like(wob),
            pltpu.VMEM((nh * _ROWS, dh), _F32),
            pltpu.VMEM((nb * nh, dh), _F32),
            pltpu.VMEM((nh, _ROWS, dh), _F32),
            pltpu.VMEM((dc // 128, nh * _ROWS, 128), _F32),
            pltpu.VMEM((nb, nh, dc), _F32),
            pltpu.VMEM((sk // _KC, nh, _KC), _F32),
            pltpu.VMEM((_ROWS, _BLOCK), _F32),
            pltpu.VMEM((max(dm, dc) * _ROWS, dh), _F32),
        ],
        compiler_params=pltpu.CompilerParams(vmem_limit_bytes=100 * 1024 * 1024),
        name="mha_cla_decode",
    )(*operands)
    return out.reshape(nb, sq, 2 * dm)
```
